```python
import jax
import jax.numpy as jnp

def _softmax(x, axis=-1):
    return jax.nn.softmax(x, axis=axis)
def _gelu(x):
    return jax.nn.gelu(x, approximate=True)
def _silu(x):
    return jax.nn.silu(x)
def _sigmoid(x):
    return jax.nn.sigmoid(x)
def _layernorm(x, axis=-1, eps=1e-5):
    m = jnp.mean(x, axis=axis, keepdims=True)
    v = jnp.var(x, axis=axis, keepdims=True)
    return (x - m) / jnp.sqrt(v + eps)
def _scatter_add(tgt, idx, src, axis=0):
    return tgt.at[idx].add(src)
def _segment_sum(src, seg, n):
    return jax.ops.segment_sum(src, seg, n)
class _Rng:
    def __init__(self, key):
        self._k = key
    def _next(self):
        self._k, sub = jax.random.split(self._k)
        return sub
    def normal(self, shape):
        return jax.random.normal(self._next(), shape, dtype=jnp.bfloat16)
    def randint(self, lo, hi, shape):
        return jax.random.randint(self._next(), shape, lo, hi, dtype=jnp.int32)
    def uniform(self, shape, lo=0.0, hi=1.0):
        return jax.random.uniform(self._next(), shape, jnp.bfloat16, lo, hi)
    def permutation(self, n):
        return jax.random.permutation(self._next(), n)


kernel_name = 'standalone__layernorm_linear__sampling'

def setup_inputs():
    _rng = _Rng(jax.random.key(int.from_bytes(__import__("os").urandom(4), "little")))
    _w = (lambda a: (lambda t: t.astype(jnp.bfloat16) if jnp.issubdtype(t.dtype, jnp.floating) else t)(jnp.asarray(a)))
    B, S, D = 1024, 32, 576
    return {
        "x": _w((lambda *s: _rng.normal(s) * 0.05)(B, S, D)),
        "g": _w((lambda *s: _rng.normal(s) * 0.05)(D) + 1.0),
        "b": _w((lambda *s: _rng.normal(s) * 0.05)(D)),
        "w": _w((lambda *s: _rng.normal(s) * 0.05)(D, D)),
    }

def reference(x, g, b, w):
    return (_layernorm(x, axis=-1) * g + b) @ w
```

```python
import jax
import jax.numpy as jnp
import jax.experimental.pallas as pl
import jax.experimental.pallas.tpu as pltpu

EPS = 1e-5


def _kernel(x_ref, g_ref, b_ref, wt_ref, o_ref):
    x = x_ref[0].astype(jnp.float32)
    d = x.shape[0]
    m = jnp.sum(x, axis=0, keepdims=True) * (1.0 / d)
    xc = x - m
    v = jnp.sum(xc * xc, axis=0, keepdims=True) * (1.0 / d)
    r = jax.lax.rsqrt(v + EPS)
    y = xc * r * g_ref[...].astype(jnp.float32) + b_ref[...].astype(jnp.float32)
    o_ref[0] = jnp.dot(
        wt_ref[...], y.astype(jnp.bfloat16), preferred_element_type=jnp.float32
    ).astype(o_ref.dtype)


@jax.jit
def pallas_standalone__layernorm_linear__sampling_kernel(x, g, b, w):
    B, S, D = x.shape
    xt = jnp.transpose(x, (1, 2, 0))
    wt = w.T
    TM = B
    out = pl.pallas_call(
        _kernel,
        grid=(S, B // TM),
        in_specs=[
            pl.BlockSpec((1, D, TM), lambda s, j: (s, 0, j)),
            pl.BlockSpec((D, 1), lambda s, j: (0, 0)),
            pl.BlockSpec((D, 1), lambda s, j: (0, 0)),
            pl.BlockSpec((D, D), lambda s, j: (0, 0)),
        ],
        out_specs=pl.BlockSpec((1, D, TM), lambda s, j: (s, 0, j)),
        out_shape=jax.ShapeDtypeStruct((S, D, B), x.dtype),
        compiler_params=pltpu.CompilerParams(
            dimension_semantics=("parallel", "parallel"),
            vmem_limit_bytes=64 * 1024 * 1024,
        ),
    )(xt, g.reshape(D, 1), b.reshape(D, 1), wt)
    return jnp.transpose(out, (2, 0, 1))
```

```python
import functools

import jax
import jax.numpy as jnp
import jax.experimental.pallas as pl
import jax.experimental.pallas.tpu as pltpu

EPS = 1e-5
F32 = jnp.float32
BF16 = jnp.bfloat16
U32 = jnp.uint32

G = 16
KP = 192
KG = 64
T = 128
NH = 288
SEG = 32
NSEG = NH // SEG
PS = KP // 2
PR = KG // 2
PROWS = 7 * PS + 6 * PR
PRODS = [(0, []), (1, [5]), (2, [4]), (3, [2]), (4, [3]), (5, [1]), (6, [0]),
         (None, [1, 4]), (None, [0, 2]), (None, [3, 5])]
NPIECE = 24
STAT_STEPS = [2] * 12 + [1] * 12


def _dot(a, b):
    return jnp.dot(a, b, preferred_element_type=F32)


def _pk(v):
    return pltpu.bitcast(v.astype(BF16), U32)


def _pk16(lo, hi):
    return pltpu.pack_elementwise([lo, hi], packed_dtype=BF16)


def _upk(v):
    return pltpu.bitcast(v, BF16)


def _bits(v):
    return pltpu.bitcast(v, U32)


def _link(v, zero):
    return pltpu.bitcast(_bits(v) | zero, F32)


def _prep_w(wbuf, g_ref, b_ref, a_ref, bias_ref):
    D = wbuf.shape[0]
    g = g_ref[...].astype(F32).reshape(1, D)
    b = b_ref[...].astype(F32).reshape(1, D)
    row = jax.lax.broadcasted_iota(jnp.int32, (128, D), 0)
    gb = jnp.where(row == 0, g, jnp.where(row == 1, b, 0.0)).T
    w = wbuf[...].astype(F32)
    wx = jnp.concatenate([w[:, :512], jnp.concatenate([w[:, 512:], gb[:, :64]], axis=1)], axis=1)
    wx = wx.reshape(D // 16, 16, 640)
    wp = pltpu.pack_elementwise([wx[:, :8], wx[:, 8:]], packed_dtype=BF16).reshape(D // 2, 640)
    wt = _upk(wp).astype(F32).T
    gp = wt[D:D + 1]
    bp = wt[D + 1:D + 2]
    wt = wt[:D]
    wg = wt * gp
    a1 = wg[:NH]
    a2 = wg[NH:]
    a11, a12, a21, a22 = a1[:, :KP], a1[:, KP:2 * KP], a2[:, :KP], a2[:, KP:2 * KP]
    o = 2 * KP
    a1A, a1B, a1C = a1[:, o:o + KG], a1[:, o + KG:o + 2 * KG], a1[:, o + 2 * KG:]
    a2A, a2B, a2C = a2[:, o:o + KG], a2[:, o + KG:o + 2 * KG], a2[:, o + 2 * KG:]

    def cat(*xs):
        return jnp.concatenate(xs, axis=1)

    z = jnp.zeros((NH, KG), F32)
    a_ref[0] = _pk(cat(a11 + a22, z))
    a_ref[1] = _pk(cat(a21 + a22, a2C - a1C))
    a_ref[2] = _pk(cat(a11, a2C))
    a_ref[3] = _pk(cat(a22, a1B))
    a_ref[4] = _pk(cat(a11 + a12, a1B - a2B))
    a_ref[5] = _pk(cat(a21 - a11, a2A))
    a_ref[6] = _pk(cat(a12 - a22, a1A))
    a_ref[7] = _pk(cat(a1A, a1C - a2C, z, z))
    a_ref[8] = _pk(cat(a2A, a2B - a1B, z, z))
    a_ref[9] = _pk(cat(-a2B, a1C, z, z))
    bias = jnp.sum(wt * bp, axis=1, keepdims=True)
    bias_ref[...] = jnp.broadcast_to(bias, bias_ref.shape)


class _Stats:
    def __init__(self, x_view):
        self.x = x_view
        self.p0 = jnp.broadcast_to(x_view[0:G, :].astype(F32)[0:1], (8, 2 * T))
        self.p = self.p0
        self.s = None
        self.q = None
        self.k = 0

    def step(self, n):
        for _ in range(n):
            x = self.x[self.k * G:(self.k + 1) * G, :].astype(F32)
            for h in range(2):
                d = x[8 * h:8 * h + 8] - self.p
                self.s = d if self.s is None else self.s + d
                self.q = d * d if self.q is None else self.q + d * d
            self.k += 1

    def finish(self):
        D = self.x.shape[0]
        s = jnp.sum(self.s, axis=0, keepdims=True) * (1.0 / D)
        q = jnp.sum(self.q, axis=0, keepdims=True) * (1.0 / D)
        var = jnp.maximum(q - s * s, 0.0)
        return self.p0[0:1] + s, jax.lax.rsqrt(var + EPS)


def _norm_tile(x_view, p_ref, cur, nxt_view, ticks):
    m, r = [jnp.broadcast_to(v, (8, 2 * T)) for v in cur]
    st = _Stats(nxt_view)
    g2 = G // 2

    def add(a, b):
        return a[0] + b[0], a[1] + b[1]

    def sub(a, b):
        return a[0] - b[0], a[1] - b[1]

    for k in range(NPIECE):
        mm = m
        if ticks is not None:
            zz = jnp.concatenate([ticks[k], ticks[k]], axis=1)
            st.p = _link(st.p0, zz)
            mm = _link(m, zz)

        def nrm(r0, mm=mm):
            x = x_view[r0:r0 + G, :].astype(F32)
            lo = (x[:8] - mm) * r
            hi = (x[8:] - mm) * r
            return (lo[:, :T], hi[:, :T]), (lo[:, T:], hi[:, T:])

        st.step(STAT_STEPS[k])
        if k < 12:
            b11, b12 = nrm(k * G)
            b21, b22 = nrm(KP + k * G)
            vals = [add(b11, b22), b11, sub(b12, b22), sub(b21, b11), b22, add(b11, b12), add(b21, b22)]
            for i, v in enumerate(vals):
                q0 = i * PS + k * g2
                p_ref[q0:q0 + g2, :] = _pk16(*v)
        else:
            kk = k - 12
            grp, j = kk // 4, kk % 4
            b1, b2 = nrm(2 * KP + kk * G)
            vals = [(b1, b2), (add(b1, b2), b2), (add(b1, b2), b1)][grp]
            for i, v in enumerate(vals):
                q0 = 7 * PS + (2 * grp + i) * PR + j * g2
                p_ref[q0:q0 + g2, :] = _pk16(*v)
    return st.finish()


def _mm_tile(p_ref, a_ref, bias_ref, obuf, s, cols):
    m = []
    for i, (si, rems) in enumerate(PRODS):
        parts = [] if si is None else [p_ref[si * PS:(si + 1) * PS, :]]
        parts += [p_ref[7 * PS + rb * PR:7 * PS + (rb + 1) * PR, :] for rb in rems]
        rhs = _upk(jnp.concatenate(parts, axis=0) if len(parts) > 1 else parts[0])
        m.append(_dot(_upk(a_ref[i, :, :rhs.shape[0]]), rhs))
    t4 = m[3] + m[9]
    t3 = m[2] - m[9]
    b1 = bias_ref[:NH, :]
    b2 = bias_ref[NH:, :]
    c11 = m[0] + t4 - m[4] + m[6] + b1
    c12 = t3 + m[4] + m[7] + b1
    c21 = m[1] + t4 + m[8] + b2
    c22 = m[0] - m[1] + t3 + m[5] + b2
    obuf[2 * s, :, :, cols] = jnp.concatenate([c11, c12], axis=1).astype(BF16).reshape(NSEG, SEG, 2 * T)
    obuf[2 * s + 1, :, :, cols] = jnp.concatenate([c21, c22], axis=1).astype(BF16).reshape(NSEG, SEG, 2 * T)
    return m


def _tick_schedule(frac):
    first_in_round = [0, 2, 4, 6]
    out = []
    for k in range(NPIECE):
        t = 4.25 * NH * frac * k / NPIECE
        out.append((first_in_round[int(t // NH)], int(t % NH) // 8 * 8))
    return out


def _body(x_hbm, g_ref, b_ref, w_hbm, o_hbm, xbuf, obuf, wbuf, a_ref, bias_ref, pa, pb, z_ref,
          isem, osem, *, first_write):
    S, D, B = x_hbm.shape
    W2 = 2 * T
    NT = B // W2
    HB = B // 2
    NBIG = (S - 2) // 2
    sched = _tick_schedule(0.8)

    def rd_half(s, h, k):
        return pltpu.make_async_copy(
            x_hbm.at[s, :, pl.ds(h * HB, HB)], xbuf.at[s, :, pl.ds(h * HB, HB)], isem.at[k])

    def rd_pair(i):
        return pltpu.make_async_copy(
            x_hbm.at[pl.ds(2 + 2 * i, 2)], xbuf.at[pl.ds(2 + 2 * i, 2)], isem.at[4 + i])

    def wr(h0, n, j):
        return pltpu.make_async_copy(obuf.at[pl.ds(h0, n), j], o_hbm.at[pl.ds(h0, n), j], osem.at[0])

    def wr_half(s, h):
        return pltpu.make_async_copy(
            obuf.at[pl.ds(2 * s, 2), :, :, pl.ds(h * HB, HB)],
            o_hbm.at[pl.ds(2 * s, 2), :, :, pl.ds(h * HB, HB)], osem.at[0])

    def tile(s, t):
        return xbuf.at[s, :, pl.ds(t * W2, W2)]

    wcp = pltpu.make_async_copy(w_hbm, wbuf, isem.at[4 + NBIG])
    wcp.start()
    for k in range(4):
        rd_half(k // 2, k % 2, k).start()
    for i in range(NBIG):
        rd_pair(i).start()
    wcp.wait()
    _prep_w(wbuf, g_ref, b_ref, a_ref, bias_ref)
    z_ref[...] = jnp.zeros(z_ref.shape, U32)
    rd_half(0, 0, 0).wait()
    st0 = _Stats(tile(0, 0))
    st0.step(D // G)
    st = _norm_tile(tile(0, 0), pa, st0.finish(), tile(0, 1), None)

    def tiles(st, s, t0, nt, dyn):
        z = z_ref[...]
        for u in range(nt):
            pc, pn = (pa, pb) if u % 2 == 0 else (pb, pa)
            if dyn:
                def view(tt):
                    tt = jnp.minimum(tt, S * NT - 1)
                    return xbuf.at[tt // NT, :, pl.ds(pl.multiple_of((tt % NT) * W2, W2), W2)]

                tau = s * NT + t0 + u
                v1, v2 = view(tau + 1), view(tau + 2)
                ms = _mm_tile(pc, a_ref, bias_ref, obuf, s, pl.ds(pl.multiple_of((t0 + u) * W2, W2), W2))
            else:
                ss, t = s + (t0 + u) // NT, (t0 + u) % NT
                v1 = tile(ss + (t + 1) // NT, (t + 1) % NT)
                v2 = tile(ss + (t + 2) // NT, (t + 2) % NT)
                ms = _mm_tile(pc, a_ref, bias_ref, obuf, ss, pl.ds(t * W2, W2))
            st = _norm_tile(v1, pn, st, v2, [_bits(ms[i][r:r + 8]) & z for i, r in sched])
        return st

    def phase(ph, st):
        def small(j, st):
            @pl.when(ph == 0)
            def _():
                rd_half((j + 1) // 2, (j + 1) % 2, j + 1).wait()

            st = tiles(st, ph * (S - 1), 2 * j, 2, True)

            @pl.when(ph == 1)
            def _():
                wr_half(S - 1, j).start()

            return st

        st = jax.lax.fori_loop(0, 2, small, st)

        def big(i, st):
            @pl.when(i == 0)
            def _():
                rd_half(1, 1, 3).wait()

            rd_pair(i).wait()

            @pl.when(i == first_write)
            def _():
                for j in range(NSEG):
                    wr(0, 2 * (2 * first_write + 1), j).start()

            @pl.when(i > first_write)
            def _():
                for j in range(NSEG):
                    wr(2 * (2 * i - 1), 4, j).start()

            return tiles(st, 1 + 2 * i, 0, 2 * NT, False)

        st = jax.lax.fori_loop(0, NBIG * (1 - ph), big, st)

        @pl.when(ph == 0)
        def _():
            for j in range(NSEG):
                wr(2 * (S - 3), 4, j).start()

        return st

    jax.lax.fori_loop(0, 2, phase, st)
    pltpu.make_async_copy(obuf, o_hbm, osem.at[0]).wait()


@jax.jit
def pallas_standalone__layernorm_linear__sampling_kernel(x, g, b, w):
    B, S, D = x.shape
    xt = jnp.transpose(x, (1, 2, 0))
    oshape = (2 * S, NSEG, SEG, B)
    out = pl.pallas_call(
        functools.partial(_body, first_write=7),
        in_specs=[
            pl.BlockSpec(memory_space=pl.ANY),
            pl.BlockSpec(memory_space=pltpu.VMEM),
            pl.BlockSpec(memory_space=pltpu.VMEM),
            pl.BlockSpec(memory_space=pl.ANY),
        ],
        out_specs=pl.BlockSpec(memory_space=pl.ANY),
        out_shape=jax.ShapeDtypeStruct(oshape, x.dtype),
        scratch_shapes=[
            pltpu.VMEM((S, D, B), BF16),
            pltpu.VMEM(oshape, BF16),
            pltpu.VMEM((D, D), BF16),
            pltpu.VMEM((10, NH // 2, 256), U32),
            pltpu.VMEM((D, T), F32),
            pltpu.VMEM((PROWS, T), U32),
            pltpu.VMEM((PROWS, T), U32),
            pltpu.VMEM((8, T), U32),
            pltpu.SemaphoreType.DMA((32,)),
            pltpu.SemaphoreType.DMA((1,)),
        ],
        compiler_params=pltpu.CompilerParams(
            vmem_limit_bytes=110 * 1024 * 1024, disable_bounds_checks=True),
    )(xt, g, b, w)
    return jnp.transpose(out.reshape(S, D, B), (2, 0, 1))
```

```python
import functools
import jax
import jax.numpy as jnp
import jax.experimental.pallas as pl
import jax.experimental.pallas.tpu as pltpu

EPS = 1e-5
F32 = jnp.float32
BF16 = jnp.bfloat16
U32 = jnp.uint32
D = 576
G = 16
T = 128
W2 = 2 * T
NH = 288
SEG = 32
NSEG = NH // SEG
PROWS = 7 * 128 + 64
SP, SM = 7 * 128, 7 * 128 + 32


def _pb(i, lo, hi):
    return ((i - 1) * 128 + lo // 2, (hi - lo) // 2)


PASSES = {
    'I': [_pb(1, 0, 96), _pb(1, 224, 256)],
    'Z': [_pb(1, 128, 224), _pb(1, 96, 128)],
    'se1': [_pb(4, 0, 128)], 'de1': [_pb(4, 128, 256)],
    'se2': [_pb(3, 0, 128)], 'de2': [_pb(3, 128, 256)],
    'e1s': [(SP, 32), _pb(5, 96, 128), _pb(5, 224, 256)],
    'e2s': [(SP, 32), _pb(2, 96, 128), _pb(2, 224, 256)],
    'e1d': [_pb(5, 0, 96), (SM, 16), _pb(5, 128, 224), (SM + 16, 16)],
    'e2d': [_pb(2, 0, 96), (SM, 16), _pb(2, 128, 224), (SM + 16, 16)],
    'e11': [_pb(7, 0, 256)], 'e22': [_pb(6, 0, 256)],
}
SIGMA = {'I': (1, 0, 0, 1), 'Z': (1, 0, 0, -1), 'se1': (1, 0, 1, 0), 'de1': (1, 0, -1, 0), 'se2': (0, 1, 0, 1),
         'de2': (0, 1, 0, -1), 'e1s': (1, 1, 0, 0), 'e1d': (1, -1, 0, 0), 'e2s': (0, 0, 1, 1), 'e2d': (0, 0, 1, -1),
         'e11': (1, 0, 0, 0), 'e22': (0, 0, 0, 1)}
ASLOT = {'I': 0, 'Z': 1, 'se1': 2, 'de1': 3, 'se2': 4, 'de2': 5, 'e1s': 6, 'e2s': 7,
         'e1d': 8, 'e2d': 10, 'e11': 12, 'e22': 14}
PLANS = {
    'a': [['I', 'se1', 'de1', 'e2s'], ['e1d', 'e11'], ['Z', 'se2', 'de2', 'e1s'], ['e2d', 'e22']],
    'b': [['e1d', 'e11'], ['I', 'se1', 'de1', 'e2s'], ['Z', 'se2', 'de2', 'e1s'], ['e2d', 'e22']],
    'c': [['I', 'se1', 'de1', 'e2s'], ['Z', 'se2', 'de2', 'e1s'], ['e1d', 'e11'], ['e2d', 'e22']],
}
NPIECE = 20
STAT_STEPS = [2] * 16 + [1] * 4
BLOCKS = [[(0, 128)], [(128, 128)], [(256, 128)], [(384, 128)], [(512, 64), (544, 32), (512, 32)]]


def _dot(a, b):
    return jnp.dot(a, b, preferred_element_type=F32)


def _pk16(lo, hi):
    return pltpu.pack_elementwise([lo, hi], packed_dtype=BF16)


def _upk(v):
    return pltpu.bitcast(v, BF16)


def _bits(v):
    return pltpu.bitcast(v, U32)


def _link(v, zero):
    return pltpu.bitcast(_bits(v) | zero, F32)


def _lane_arrange(v_ref):
    v8 = jnp.broadcast_to(v_ref[...].astype(F32).reshape(1, D), (8, D))
    lane = jax.lax.broadcasted_iota(jnp.int32, (8, 128), 1)
    perm = (lane & ~15) | ((lane & 15) >> 1) | ((lane & 1) << 3)
    out = [jnp.take_along_axis(v8[:, 128 * i:128 * (i + 1)], perm, axis=1) for i in range(4)]
    last = jnp.concatenate([v8[:, 512:], v8[:, 512:]], axis=1)
    idx = jnp.where(lane < 64, perm, jnp.where(lane < 96, perm - 32, perm - 96))
    out.append(jnp.take_along_axis(last, idx, axis=1))
    return out


def _prep_w1(w_ref, wt_ref):
    for c in (0, 2, 1, 3, 4):
        wd = min(128, D - 128 * c)
        for bi, blk in enumerate(BLOCKS):
            rows = []
            for (st, ln) in blk:
                w = w_ref[st:st + ln, 128 * c:128 * c + wd].astype(F32).reshape(ln // 16, 16, wd)
                rows.append(_pk16(w[:, :8], w[:, 8:]).reshape(ln // 2, wd))
            wp = jnp.concatenate(rows, axis=0) if len(rows) > 1 else rows[0]
            wt_ref[bi, 64 * c:64 * c + wd // 2, :] = _bits(_upk(wp).T)


def _prep_w2(g_ref, b_ref, wt_ref, a_ref, bias_ref):
    gt = _lane_arrange(g_ref)
    bt = _lane_arrange(b_ref)
    lane = jax.lax.broadcasted_iota(jnp.int32, (8, 128), 1)
    bt[4] = jnp.where(lane < 64, bt[4], 0.0)
    gt[4] = gt[4] * 0.5

    def s96(a, b):
        return jnp.where(lane < 96, a, b)

    for j in range(NH // 16):
        res = []
        for par in range(2):
            raw = [[pltpu.unpack_elementwise(wt_ref[bi, 8 * (j + h * 18):8 * (j + h * 18) + 8, :], index=par,
                                             packed_dtype=BF16, unpacked_dtype=F32) for bi in range(5)]
                   for h in range(2)]
            for h in range(2):
                bs = raw[h][0] * bt[0]
                for bi in range(1, 5):
                    bs = bs + raw[h][bi] * bt[bi]
                bias_ref[pl.ds(16 * (j + h * 18) + par, 8, stride=2), :] = jnp.broadcast_to(
                    jnp.sum(bs, axis=1, keepdims=True), (8, 128))
            n1 = [raw[0][bi] * gt[bi] for bi in range(5)]
            n2 = [raw[1][bi] * gt[bi] for bi in range(5)]
            a1x, a1y = n1[0] + n2[1], n1[2] - n2[3]
            s5x, s5y = n1[0] + n1[1], n1[2] + n1[3]
            s2x, s2y = n2[0] + n2[1], n2[2] + n2[3]
            a6x, a6y = n2[0] - n1[0], n2[2] + n1[2]

            def es(sv, sx, sy):
                return jnp.where(lane < 64, sv, s96(pltpu.roll(sx, 96, 1), sy))

            res.append([
                s96(a1x, a1y), s96(a1y, a1x), n2[1], -n2[3], n1[0], n1[2],
                es(n1[4], s5x, s5y), es(n2[4], s2x, s2y),
                s96(-s5x, n1[4]), s96(-s5y, pltpu.roll(n1[4], 32, 1)),
                s96(s2x, n2[4]), s96(s2y, pltpu.roll(n2[4], 32, 1)),
                n1[1] - n2[1], n1[3] + n2[3],
                s96(a6x, -a6x), s96(a6y, -a6y),
            ])
        for i in range(16):
            a_ref[i, 8 * j:8 * j + 8, :] = _pk16(res[0][i], res[1][i])


class _Stats:
    def __init__(self, x_view):
        self.x = x_view
        self.p0 = jnp.broadcast_to(x_view[0:G, :].astype(F32)[0:1], (8, W2))
        self.p = self.p0
        self.s = None
        self.q = None
        self.k = 0

    def step(self, n):
        for _ in range(n):
            x = self.x[self.k * G:(self.k + 1) * G, :].astype(F32)
            for h in range(2):
                d = x[8 * h:8 * h + 8] - self.p
                self.s = d if self.s is None else self.s + d
                self.q = d * d if self.q is None else self.q + d * d
            self.k += 1

    def finish(self):
        s = jnp.sum(self.s, axis=0, keepdims=True) * (1.0 / D)
        q = jnp.sum(self.q, axis=0, keepdims=True) * (1.0 / D)
        var = jnp.maximum(q - s * s, 0.0)
        return self.p0[0:1] + s, jax.lax.rsqrt(var + EPS)


def _norm_tile(x_view, p_ref, cur, nxt_view, ticks):
    m, r = [jnp.broadcast_to(v, (8, W2)) for v in cur]
    st = _Stats(nxt_view)

    def add(a, b):
        return a[0] + b[0], a[1] + b[1]

    def sub(a, b):
        return a[0] - b[0], a[1] - b[1]

    for k in range(NPIECE):
        mm = m
        if ticks is not None:
            zz = jnp.concatenate([ticks[k], ticks[k]], axis=1)
            st.p = _link(st.p0, zz)
            mm = _link(m, zz)

        def nrm(r0, mm=mm):
            x = x_view[r0:r0 + G, :].astype(F32)
            lo = (x[:8] - mm) * r
            hi = (x[8:] - mm) * r
            return (lo[:, :T], hi[:, :T]), (lo[:, T:], hi[:, T:])

        st.step(STAT_STEPS[k])
        if k < 16:
            r0 = (k // 8) * 256 + (k % 8) * G
            b11, b12 = nrm(r0)
            b21, b22 = nrm(r0 + 128)
            pm = add if k % 8 < 6 else sub
            vals = [pm(b11, b22), b11, sub(b12, b22), sub(b21, b11), b22, pm(b11, b12), pm(b21, b22)]
            for i, v in enumerate(vals):
                q0 = i * 128 + k * 8
                p_ref[q0:q0 + 8, :] = _pk16(*v)
        else:
            kk = k - 16
            b1, b2 = nrm(512 + kk * G)
            p_ref[SP + kk * 8:SP + kk * 8 + 8, :] = _pk16(*add(b1, b2))
            p_ref[SM + kk * 8:SM + kk * 8 + 8, :] = _pk16(*sub(b1, b2))
    return st.finish()


def _mm_tile(p_ref, a_ref, bias_ref, obuf, s, cols, plan):
    m = {}
    acc = [None] * 4
    for rnd in plan:
        for nm in rnd:
            parts = [p_ref[q0:q0 + n, :] for q0, n in PASSES[nm]]
            rhs = _upk(jnp.concatenate(parts, axis=0) if len(parts) > 1 else parts[0])
            sl = ASLOT[nm]
            lhs = a_ref[sl] if rhs.shape[0] == 128 else jnp.concatenate([a_ref[sl], a_ref[sl + 1]], axis=1)
            m[nm] = _dot(_upk(lhs), rhs)
        for q in range(4):
            terms = [(nm, SIGMA[nm][q]) for nm in rnd if SIGMA[nm][q]]
            if not terms:
                continue
            s0 = terms[0][1]
            val = m[terms[0][0]]
            for nm, sg in terms[1:]:
                val = val + m[nm] if sg * s0 > 0 else val - m[nm]
            prev = acc[q] if acc[q] is not None else (bias_ref[:NH, :] if q < 2 else bias_ref[NH:, :])
            acc[q] = prev + val if s0 > 0 else prev - val
    obuf[2 * s, :, :, cols] = jnp.concatenate(acc[:2], axis=1).astype(BF16).reshape(NSEG, SEG, W2)
    obuf[2 * s + 1, :, :, cols] = jnp.concatenate(acc[2:], axis=1).astype(BF16).reshape(NSEG, SEG, W2)
    return m


def _ticks(m, z, plan, span):
    out = []
    for k in range(NPIECE):
        t = span * k / NPIECE
        out.append(_bits(m[plan[int(t // NH)][0]][int(t % NH) // 8 * 8:][:8]) & z)
    return out


def _body(x_hbm, g_hbm, b_hbm, w_hbm, o_hbm, xbuf, obuf, wbuf, gbuf, bbuf, wt_ref, a_ref, bias_ref, pa, pb, z_ref,
          isem, osem, *, U, head, first_write, spans, plan, nodma):
    S, _, B = x_hbm.shape
    NT = B // W2
    hs = sum(head) // NT
    NIT = (S - hs) // U
    plan = PLANS[plan]

    def rd_cols(t0, n, k):
        return pltpu.make_async_copy(
            x_hbm.at[0, :, pl.ds(t0 * W2, n * W2)], xbuf.at[0, :, pl.ds(t0 * W2, n * W2)], isem.at[k])

    def rd(s0, n, k):
        return pltpu.make_async_copy(x_hbm.at[pl.ds(s0, n)], xbuf.at[pl.ds(s0, n)], isem.at[k])

    def wr(h0, n, j):
        return pltpu.make_async_copy(obuf.at[pl.ds(h0, n), j], o_hbm.at[pl.ds(h0, n), j], osem.at[0])

    def wr_cols(s, c0, w):
        return pltpu.make_async_copy(
            obuf.at[pl.ds(2 * s, 2), :, :, pl.ds(c0, w)], o_hbm.at[pl.ds(2 * s, 2), :, :, pl.ds(c0, w)], osem.at[0])

    def tile(s, t):
        return xbuf.at[s, :, pl.ds(t * W2, W2)]

    pre = [pltpu.make_async_copy(w_hbm, wbuf, isem.at[0]),
           pltpu.make_async_copy(g_hbm, gbuf, isem.at[1]),
           pltpu.make_async_copy(b_hbm, bbuf, isem.at[2]),
           rd_cols(0, 2, 3), rd_cols(2, 2, 4)]
    k = 5
    head_waits = [[pre[4]]]
    have = 1
    pos = head[0]
    for n in head[1:]:
        need = (pos + n + 1) // NT + 1
        cps = []
        if need > have:
            cps.append(rd(have, need - have, k)); k += 1
            have = need
        head_waits.append(cps)
        pos += n
    assert have == hs + 1
    k0 = k
    loop_rd = lambda i: rd(hs + 1 + U * i, U, k0 + i)
    last_rd = rd(S - U + 1, U - 1, k0 + NIT - 1)
    allrd = pre + [c for cs in head_waits[1:] for c in cs]
    if not nodma:
        allrd += [loop_rd(i) for i in range(NIT - 1)] + [last_rd]
    for cp in allrd:
        cp.start()

    pre[0].wait()
    _prep_w1(wbuf, wt_ref)
    pre[1].wait(); pre[2].wait(); pre[3].wait()
    _prep_w2(gbuf, bbuf, wt_ref, a_ref, bias_ref)
    z_ref[...] = jnp.zeros(z_ref.shape, U32)
    st0 = _Stats(tile(0, 0))
    st0.step(D // G)
    st = _norm_tile(tile(0, 0), pa, st0.finish(), tile(0, 1), None)

    def block(st, s0, t0, n, after=None):
        z = z_ref[...]
        for u in range(n):
            pc, pn = (pa, pb) if u % 2 == 0 else (pb, pa)
            ds, t = divmod(t0 + u, NT)

            def view(tt):
                d2, t2 = divmod(tt, NT)
                s2 = s0 + d2
                if not isinstance(s2, int) and d2 == U:
                    s2 = jnp.minimum(s2, S - 1)
                return tile(s2, t2)

            m = _mm_tile(pc, a_ref, bias_ref, obuf, s0 + ds, pl.ds(t * W2, W2), plan)
            span = spans[0] if u < n - 1 else spans[1]
            st = _norm_tile(view(t0 + u + 1), pn, st, view(t0 + u + 2), _ticks(m, z, plan, span))
            if after is not None:
                after(s0 + ds, ds, t)
        return st

    pos = 0
    for n, cps in zip(head, head_waits):
        for cp in cps:
            cp.wait()
        st = block(st, 0, pos, n)
        pos += n

    def it(i, st):
        s0 = hs + i * U
        last = i == NIT - 1
        if nodma:
            return block(st, s0, 0, U * NT, None)

        @pl.when(jnp.logical_not(last))
        def _():
            loop_rd(i).wait()

        @pl.when(last)
        def _():
            last_rd.wait()

        @pl.when(i == first_write)
        def _():
            for j in range(NSEG):
                wr(0, 2 * (hs + U * first_write), j).start()

        @pl.when(i > first_write)
        def _():
            for j in range(NSEG):
                wr(2 * (s0 - U), 2 * U, j).start()

        def after(s, ds, t):
            if ds < U - 1 and t == NT - 1:
                @pl.when(last)
                def _():
                    wr_cols(s, 0, B).start()
            elif ds == U - 1:
                @pl.when(last)
                def _():
                    wr_cols(s, t * W2, W2).start()

        return block(st, s0, 0, U * NT, after)

    jax.lax.fori_loop(0, NIT, it, st)
    if nodma:
        wr(0, 1, 0).start(); wr(0, 1, 0).wait()
    else:
        pltpu.make_async_copy(obuf, o_hbm, osem.at[0]).wait()


@jax.jit
def pallas_standalone__layernorm_linear__sampling_kernel(x, g, b, w):
    B, S, _ = x.shape
    xt = jnp.transpose(x, (1, 2, 0))
    oshape = (2 * S, NSEG, SEG, B)
    out = pl.pallas_call(
        functools.partial(_body, U=2, head=(2, 2, 4), first_write=6, spans=(930, 1050), plan='a', nodma=False),
        in_specs=[pl.BlockSpec(memory_space=pl.ANY)] * 4,
        out_specs=pl.BlockSpec(memory_space=pl.ANY),
        out_shape=jax.ShapeDtypeStruct(oshape, x.dtype),
        scratch_shapes=[
            pltpu.VMEM((S, D, B), BF16),
            pltpu.VMEM(oshape, BF16),
            pltpu.VMEM((D, D), BF16),
            pltpu.VMEM((D,), BF16),
            pltpu.VMEM((D,), BF16),
            pltpu.VMEM((5, D // 2, 128), U32),
            pltpu.VMEM((16, NH // 2, 128), U32),
            pltpu.VMEM((D, T), F32),
            pltpu.VMEM((PROWS, T), U32),
            pltpu.VMEM((PROWS, T), U32),
            pltpu.VMEM((8, T), U32),
            pltpu.SemaphoreType.DMA((32,)),
            pltpu.SemaphoreType.DMA((1,)),
        ],
        compiler_params=pltpu.CompilerParams(
            vmem_limit_bytes=110 * 1024 * 1024, disable_bounds_checks=True),
    )(xt, g, b, w)
    return jnp.transpose(out.reshape(S, D, B), (2, 0, 1))
```

```python
import functools

import jax
import jax.numpy as jnp
import jax.experimental.pallas as pl
import jax.experimental.pallas.tpu as pltpu

EPS = 1e-5
F32 = jnp.float32
BF16 = jnp.bfloat16
U32 = jnp.uint32

D = 576
G = 16
T = 128
W2 = 2 * T
NH = D // 2
SEG = 32
NSEG = NH // SEG
PROWS = 7 * 128 + 64
SP, SM = 7 * 128, 7 * 128 + 32


def _rows(i, lo, hi):
    return (i - 1) * 128 + lo // 2, (hi - lo) // 2


PASSES = {
    'I': [_rows(1, 0, 96), _rows(1, 224, 256)],
    'Z': [_rows(1, 128, 224), _rows(1, 96, 128)],
    'se1': [_rows(4, 0, 128)], 'de1': [_rows(4, 128, 256)],
    'se2': [_rows(3, 0, 128)], 'de2': [_rows(3, 128, 256)],
    'e1s': [(SP, 32), _rows(5, 96, 128), _rows(5, 224, 256)],
    'e2s': [(SP, 32), _rows(2, 96, 128), _rows(2, 224, 256)],
    'e1d': [_rows(5, 0, 96), (SM, 16), _rows(5, 128, 224), (SM + 16, 16)],
    'e2d': [_rows(2, 0, 96), (SM, 16), _rows(2, 128, 224), (SM + 16, 16)],
    'e11': [_rows(7, 0, 256)], 'e22': [_rows(6, 0, 256)],
}
SIGMA = {'I': (1, 0, 0, 1), 'Z': (1, 0, 0, -1), 'se1': (1, 0, 1, 0), 'de1': (1, 0, -1, 0),
         'se2': (0, 1, 0, 1), 'de2': (0, 1, 0, -1), 'e1s': (1, 1, 0, 0), 'e1d': (1, -1, 0, 0),
         'e2s': (0, 0, 1, 1), 'e2d': (0, 0, 1, -1), 'e11': (1, 0, 0, 0), 'e22': (0, 0, 0, 1)}
ASLOT = {'I': 0, 'Z': 1, 'se1': 2, 'de1': 3, 'se2': 4, 'de2': 5, 'e1s': 6, 'e2s': 7,
         'e1d': 8, 'e2d': 10, 'e11': 12, 'e22': 14}
PLAN = [['I', 'se1', 'de1', 'e2s'], ['e1d', 'e11'], ['Z', 'se2', 'de2', 'e1s'], ['e2d', 'e22']]
PLAN0 = [['se1', 'de1', 'se2', 'de2'], ['e1d', 'e11'], ['I', 'Z', 'e1s', 'e2s'], ['e2d', 'e22']]
NPIECE = 20
STAT_STEPS = [2] * 16 + [1] * 4
BLOCKS = [[(0, 128)], [(128, 128)], [(256, 128)], [(384, 128)], [(512, 64), (544, 32), (512, 32)]]


def _dot(a, b):
    return jnp.dot(a, b, preferred_element_type=F32)


def _pk16(lo, hi):
    return pltpu.pack_elementwise([lo, hi], packed_dtype=BF16)


def _upk(v):
    return pltpu.bitcast(v, BF16)


def _bits(v):
    return pltpu.bitcast(v, U32)


def _link(v, zero):
    return pltpu.bitcast(_bits(v) | zero, F32)


def _lane_arrange(v_ref):
    v8 = jnp.broadcast_to(v_ref[...].astype(F32).reshape(1, D), (8, D))
    lane = jax.lax.broadcasted_iota(jnp.int32, (8, 128), 1)
    perm = (lane & ~15) | ((lane & 15) >> 1) | ((lane & 1) << 3)
    out = [jnp.take_along_axis(v8[:, 128 * i:128 * (i + 1)], perm, axis=1) for i in range(4)]
    last = jnp.concatenate([v8[:, 512:], v8[:, 512:]], axis=1)
    idx = jnp.where(lane < 64, perm, jnp.where(lane < 96, perm - 32, perm - 96))
    out.append(jnp.take_along_axis(last, idx, axis=1))
    return out


def _transpose_w(w_ref, wt_ref, blocks):
    for bi in blocks:
        for c in range(5):
            wd = min(128, D - 128 * c)
            rows = []
            for st, ln in BLOCKS[bi]:
                w = w_ref[st:st + ln, 128 * c:128 * c + wd].astype(F32).reshape(ln // 16, 16, wd)
                rows.append(_pk16(w[:, :8], w[:, 8:]).reshape(ln // 2, wd))
            wp = jnp.concatenate(rows, axis=0) if len(rows) > 1 else rows[0]
            wt_ref[bi, 64 * c:64 * c + wd // 2, :] = _bits(_upk(wp).T)


def _prep_a(gt, wt_ref, a_ref, slots):
    lane = jax.lax.broadcasted_iota(jnp.int32, (8, 128), 1)

    def s96(a, b):
        return jnp.where(lane < 96, a, b)

    def es(sv, sx, sy):
        return jnp.where(lane < 64, sv, s96(pltpu.roll(sx, 96, 1), sy))

    for j in range(NH // 16):
        res = []
        for par in range(2):
            memo = {}

            def n(h, bi):
                if (h, bi) not in memo:
                    r0 = 8 * (j + (h - 1) * (NH // 16))
                    memo[(h, bi)] = gt[bi] * pltpu.unpack_elementwise(
                        wt_ref[bi, r0:r0 + 8, :], index=par, packed_dtype=BF16, unpacked_dtype=F32)
                return memo[(h, bi)]

            def c(h1, b1, sg, h2, b2):
                key = (h1, b1, sg, h2, b2)
                if key not in memo:
                    memo[key] = n(h1, b1) + n(h2, b2) if sg > 0 else n(h1, b1) - n(h2, b2)
                return memo[key]

            fns = [
                lambda: s96(c(1, 0, 1, 2, 1), c(1, 2, -1, 2, 3)),
                lambda: s96(c(1, 2, -1, 2, 3), c(1, 0, 1, 2, 1)),
                lambda: n(2, 1), lambda: -n(2, 3), lambda: n(1, 0), lambda: n(1, 2),
                lambda: es(n(1, 4), c(1, 0, 1, 1, 1), c(1, 2, 1, 1, 3)),
                lambda: es(n(2, 4), c(2, 0, 1, 2, 1), c(2, 2, 1, 2, 3)),
                lambda: s96(-c(1, 0, 1, 1, 1), n(1, 4)),
                lambda: s96(-c(1, 2, 1, 1, 3), pltpu.roll(n(1, 4), 32, 1)),
                lambda: s96(c(2, 0, 1, 2, 1), n(2, 4)),
                lambda: s96(c(2, 2, 1, 2, 3), pltpu.roll(n(2, 4), 32, 1)),
                lambda: c(1, 1, -1, 2, 1), lambda: c(1, 3, 1, 2, 3),
                lambda: s96(c(2, 0, -1, 1, 0), -c(2, 0, -1, 1, 0)),
                lambda: s96(c(2, 2, 1, 1, 2), -c(2, 2, 1, 1, 2)),
            ]
            res.append([fns[i]() for i in slots])
        for i, ev, od in zip(slots, *res):
            a_ref[i, 8 * j:8 * j + 8, :] = _pk16(ev, od)


class _Stats:
    def __init__(self, x_view):
        self.x = x_view
        self.p0 = jnp.broadcast_to(x_view[0:G, :].astype(F32)[0:1], (8, W2))
        self.p = self.p0
        self.s = None
        self.q = None
        self.k = 0

    def step(self, n):
        for _ in range(n):
            x = self.x[self.k * G:(self.k + 1) * G, :].astype(F32)
            for h in range(2):
                d = x[8 * h:8 * h + 8] - self.p
                self.s = d if self.s is None else self.s + d
                self.q = d * d if self.q is None else self.q + d * d
            self.k += 1

    def finish(self):
        s = jnp.sum(self.s, axis=0, keepdims=True) * (1.0 / D)
        q = jnp.sum(self.q, axis=0, keepdims=True) * (1.0 / D)
        var = jnp.maximum(q - s * s, 0.0)
        return self.p0[0:1] + s, jax.lax.rsqrt(var + EPS)


def _prep_tile(x_view, p_ref, cur, nxt_view, tick, t0, t1):
    def zz_at(t):
        z = tick(t)
        return jnp.concatenate([z, z], axis=1)

    if cur is None:
        st = _Stats(x_view)
        tm = t0 + (t1 - t0) * (0.33 if nxt_view is not None else 0.5)
        for k in range(12):
            if tick is not None:
                st.p = _link(st.p0, zz_at(t0 + (tm - t0) * k / 12))
            st.step(3)
        cur = st.finish()
        t0 = tm
    m, r = [jnp.broadcast_to(v, (8, W2)) for v in cur]
    st = None if nxt_view is None else _Stats(nxt_view)

    def add(a, b):
        return a[0] + b[0], a[1] + b[1]

    def sub(a, b):
        return a[0] - b[0], a[1] - b[1]

    for k in range(NPIECE):
        mm = m
        if tick is not None:
            zz = zz_at(t0 + (t1 - t0) * k / NPIECE)
            mm = _link(m, zz)
            if st is not None:
                st.p = _link(st.p0, zz)

        def nrm(r0, mm=mm):
            x = x_view[r0:r0 + G, :].astype(F32)
            lo = (x[:8] - mm) * r
            hi = (x[8:] - mm) * r
            return (lo[:, :T], hi[:, :T]), (lo[:, T:], hi[:, T:])

        if st is not None:
            st.step(STAT_STEPS[k])
        if k < 16:
            r0 = (k // 8) * 256 + (k % 8) * G
            b11, b12 = nrm(r0)
            b21, b22 = nrm(r0 + 128)
            pm = add if k % 8 < 6 else sub
            vals = [pm(b11, b22), b11, sub(b12, b22), sub(b21, b11), b22, pm(b11, b12), pm(b21, b22)]
            for i, v in enumerate(vals):
                q0 = i * 128 + k * 8
                p_ref[q0:q0 + 8, :] = _pk16(*v)
        else:
            kk = k - 16
            b1, b2 = nrm(512 + kk * G)
            p_ref[SP + kk * 8:SP + kk * 8 + 8, :] = _pk16(*add(b1, b2))
            p_ref[SM + kk * 8:SM + kk * 8 + 8, :] = _pk16(*sub(b1, b2))
    return None if st is None else st.finish()


def _mm_tile(p_ref, a_ref, bias_ref, obuf, s, cols, plan):
    m = {}
    acc = [None] * 4
    for rnd in plan:
        for nm in rnd:
            parts = [p_ref[q0:q0 + n, :] for q0, n in PASSES[nm]]
            rhs = _upk(jnp.concatenate(parts, axis=0) if len(parts) > 1 else parts[0])
            sl = ASLOT[nm]
            lhs = a_ref[sl] if rhs.shape[0] == 128 else jnp.concatenate([a_ref[sl], a_ref[sl + 1]], axis=1)
            m[nm] = _dot(_upk(lhs), rhs)
        for q in range(4):
            terms = [(nm, SIGMA[nm][q]) for nm in rnd if SIGMA[nm][q]]
            if not terms:
                continue
            s0 = terms[0][1]
            val = m[terms[0][0]]
            for nm, sg in terms[1:]:
                val = val + m[nm] if sg * s0 > 0 else val - m[nm]
            prev = acc[q] if acc[q] is not None else (bias_ref[:NH, :] if q < 2 else bias_ref[NH:, :])
            acc[q] = prev + val if s0 > 0 else prev - val
    obuf[2 * s, :, :, cols] = jnp.concatenate(acc[:2], axis=1).astype(BF16).reshape(NSEG, SEG, W2)
    obuf[2 * s + 1, :, :, cols] = jnp.concatenate(acc[2:], axis=1).astype(BF16).reshape(NSEG, SEG, W2)
    return m


def _write_runs(S, nhead, tpi, tau_w, lead):
    events = {}
    for k in range(S // 2 - 1):
        events.setdefault(max(tau_w + 4 * max(k - lead, 0), 8 * k + 8), []).append(4 * k)
    runs = {}
    for tau in sorted(events):
        for slot, h0 in enumerate(events[tau]):
            i, u = divmod(tau - nhead, tpi)
            lst = runs.setdefault((u, slot), [])
            if lst and lst[-1][1] == i - 1 and lst[-1][3] in (None, (h0 - lst[-1][2]) / (i - lst[-1][0])):
                i0, _, hh, _ = lst[-1]
                lst[-1] = (i0, i, hh, (h0 - hh) // (i - i0))
            else:
                lst.append((i, i, h0, None))
    return runs


def _body(x_hbm, g_hbm, b_hbm, w_hbm, o_hbm, xbuf, obuf, wbuf, gbuf, bbuf, wt_ref, a_ref, bias_ref,
          pa, pb, z_ref, isem, osem, *, U, head, tau_w, lead, spans, b0):
    S, _, B = x_hbm.shape
    NT = B // W2
    nhead = sum(head)
    hs = nhead // NT
    NIT = (S - hs) // U
    TPI = U * NT
    pbuf = (pa, pb)

    def rd_cols(s, t0, n, k):
        return pltpu.make_async_copy(
            x_hbm.at[s, :, pl.ds(t0 * W2, n * W2)], xbuf.at[s, :, pl.ds(t0 * W2, n * W2)], isem.at[k])

    def rd(s0, n, k):
        return pltpu.make_async_copy(x_hbm.at[pl.ds(s0, n)], xbuf.at[pl.ds(s0, n)], isem.at[k])

    def wr(h0, n, j):
        return pltpu.make_async_copy(obuf.at[pl.ds(h0, n), j], o_hbm.at[pl.ds(h0, n), j], osem.at[0])

    def wr_cols(s, c0, w):
        return pltpu.make_async_copy(
            obuf.at[pl.ds(2 * s, 2), :, :, pl.ds(c0, w)],
            o_hbm.at[pl.ds(2 * s, 2), :, :, pl.ds(c0, w)], osem.at[0])

    def tile(s, t):
        return xbuf.at[s, :, pl.ds(t * W2, W2)]

    first = [pltpu.make_async_copy(g_hbm, gbuf, isem.at[0]),
             pltpu.make_async_copy(b_hbm, bbuf, isem.at[0]),
             pltpu.make_async_copy(w_hbm, wbuf, isem.at[0])]
    x0 = rd_cols(0, 0, 1, 1)
    have = 1
    head_waits = []
    pos = 0
    for bi, n in enumerate(head):
        need = pos + n + (1 if bi == 0 else 2)
        if bi == len(head) - 1 or need > 2 * NT:
            need = -(-need // NT) * NT
        cps = []
        while have < need:
            s, t = divmod(have, NT)
            if t == 0 and need - have >= NT:
                ns = (need - have) // NT
                cps.append(rd(s, ns, 2 + bi))
                have += ns * NT
            else:
                nt = min(NT - t, need - have)
                cps.append(rd_cols(s, t, nt, 2 + bi))
                have += nt
        head_waits.append(cps)
        pos += n
    k0 = 2 + len(head)

    def loop_rd(i):
        return rd(hs + 1 + U * i, U, k0 + i)

    last_rd = rd(S - U + 1, U - 1, k0 + NIT - 1)
    for cp in (first + [x0] + [c for cs in head_waits for c in cs]
               + [loop_rd(i) for i in range(NIT - 1)] + [last_rd]):
        cp.start()

    for cp in first:
        cp.wait()
    _transpose_w(wbuf, wt_ref, range(5))
    brow = _dot(jnp.broadcast_to(bbuf[...].reshape(1, D), (16, D)), wbuf[...])[0:1]
    x0.wait()
    bias_ref[...] = jnp.broadcast_to(brow, (T, D)).T
    z_ref[...] = jnp.zeros(z_ref.shape, U32)
    gt = _lane_arrange(gbuf)
    gt[4] = gt[4] * 0.5
    _prep_tile(tile(0, 0), pa, None, None, None, 0, 0)
    early = [2, 3, 4, 5]
    _prep_a(gt, wt_ref, a_ref, early)

    def block(st, s0, t0, n, after=None, first=False):
        z = z_ref[...]
        for u in range(n):
            tt = t0 + u
            ds, t = divmod(tt, NT)

            def view(q):
                d2, t2 = divmod(q, NT)
                s2 = s0 + d2
                if not isinstance(s2, int) and d2 == U:
                    s2 = jnp.minimum(s2, S - 1)
                return tile(s2, t2)

            plan = PLAN0 if first else PLAN
            m = _mm_tile(pbuf[tt % 2], a_ref, bias_ref, obuf, s0 + ds, pl.ds(t * W2, W2), plan)

            def tick(tm, m=m, plan=plan):
                return _bits(m[plan[int(tm // NH)][0]][int(tm % NH) // 8 * 8:][:8]) & z

            st = _prep_tile(view(tt + 1), pbuf[(tt + 1) % 2], st, None if first else view(tt + 2), tick,
                            b0 if first else 0, spans[0] if u < n - 1 else spans[1])
            if after is not None:
                after(s0 + ds, tt)
        return st

    pos = 0
    st = None
    for bi, (n, cps) in enumerate(zip(head, head_waits)):
        for cp in cps:
            cp.wait()
        if bi == 0:
            _prep_a(gt, wt_ref, a_ref, [i for i in range(16) if i not in early])
        st = block(st, 0, pos, n, first=bi == 0)
        pos += n

    runs = _write_runs(S, nhead, TPI, tau_w, lead)

    def it(i, st):
        last = i == NIT - 1

        @pl.when(jnp.logical_not(last))
        def _():
            loop_rd(i).wait()

        @pl.when(last)
        def _():
            last_rd.wait()

        def issue(u):
            for (uu, _), lst in sorted(runs.items()):
                for i0, i1, hh, dh in lst if uu == u else []:
                    @pl.when(jnp.logical_and(i >= i0, i <= i1))
                    def _():
                        for j in range(NSEG):
                            wr(hh if dh is None else hh + dh * (i - i0), 4, j).start()

        def after(s, tt):
            if tt + 1 < TPI:
                issue(tt + 1)
            if tt == TPI - NT - 1:
                @pl.when(last)
                def _():
                    for j in range(NSEG):
                        wr(2 * s, 2, j).start()
            if tt // NT == U - 1:
                @pl.when(last)
                def _():
                    wr_cols(s, (tt % NT) * W2, W2).start()

        issue(0)
        return block(st, hs + i * U, 0, TPI, after)

    jax.lax.fori_loop(0, NIT, it, st)
    pltpu.make_async_copy(obuf, o_hbm, osem.at[0]).wait()


def _run(x, g, b, w, U=4, head=(1, 1, 2, 4, 8), tau_w=62, lead=1, spans=(930, 1050), b0=250):
    B, S, _ = x.shape
    xt = jnp.transpose(x, (1, 2, 0))
    oshape = (2 * S, NSEG, SEG, B)
    nsem = 2 + len(head) + (S - sum(head) * W2 // B) // U
    out = pl.pallas_call(
        functools.partial(_body, U=U, head=head, tau_w=tau_w, lead=lead, spans=spans, b0=b0),
        in_specs=[pl.BlockSpec(memory_space=pl.ANY)] * 4,
        out_specs=pl.BlockSpec(memory_space=pl.ANY),
        out_shape=jax.ShapeDtypeStruct(oshape, x.dtype),
        scratch_shapes=[
            pltpu.VMEM((S, D, B), BF16),
            pltpu.VMEM(oshape, BF16),
            pltpu.VMEM((D, D), BF16),
            pltpu.VMEM((D,), BF16),
            pltpu.VMEM((D,), BF16),
            pltpu.VMEM((5, D // 2, 128), U32),
            pltpu.VMEM((16, NH // 2, 128), U32),
            pltpu.VMEM((D, T), F32),
            pltpu.VMEM((PROWS, T), U32),
            pltpu.VMEM((PROWS, T), U32),
            pltpu.VMEM((8, T), U32),
            pltpu.SemaphoreType.DMA((nsem,)),
            pltpu.SemaphoreType.DMA((1,)),
        ],
        compiler_params=pltpu.CompilerParams(
            vmem_limit_bytes=110 * 1024 * 1024,
            disable_bounds_checks=True,
            disable_semaphore_checks=True,
        ),
    )(xt, g, b, w)
    return jnp.transpose(out.reshape(S, D, B), (2, 0, 1))


@jax.jit
def pallas_standalone__layernorm_linear__sampling_kernel(x, g, b, w):
    return _run(x, g, b, w)
```

```python
import functools

import jax
import jax.numpy as jnp
import jax.experimental.pallas as pl
import jax.experimental.pallas.tpu as pltpu

EPS = 1e-5
F32 = jnp.float32
BF16 = jnp.bfloat16
U32 = jnp.uint32

D = 576
G = 16
T = 128
W2 = 2 * T
NH = D // 2
SEG = 16
PROWS = 7 * 128 + 64
SP, SM = 7 * 128, 7 * 128 + 32


def _rows(i, lo, hi):
    return (i - 1) * 128 + lo // 2, (hi - lo) // 2


PASSES = {
    'I': [_rows(1, 0, 96), _rows(1, 224, 256)],
    'Z': [_rows(1, 128, 224), _rows(1, 96, 128)],
    'se1': [_rows(4, 0, 128)], 'de1': [_rows(4, 128, 256)],
    'se2': [_rows(3, 0, 128)], 'de2': [_rows(3, 128, 256)],
    'e1s': [(SP, 32), _rows(5, 96, 128), _rows(5, 224, 256)],
    'e2s': [(SP, 32), _rows(2, 96, 128), _rows(2, 224, 256)],
    'e1d': [_rows(5, 0, 96), (SM, 16), _rows(5, 128, 224), (SM + 16, 16)],
    'e2d': [_rows(2, 0, 96), (SM, 16), _rows(2, 128, 224), (SM + 16, 16)],
    'e11': [_rows(7, 0, 256)], 'e22': [_rows(6, 0, 256)],
}
SIGMA = {'I': (1, 0, 0, 1), 'Z': (1, 0, 0, -1), 'se1': (1, 0, 1, 0), 'de1': (1, 0, -1, 0),
         'se2': (0, 1, 0, 1), 'de2': (0, 1, 0, -1), 'e1s': (1, 1, 0, 0), 'e1d': (1, -1, 0, 0),
         'e2s': (0, 0, 1, 1), 'e2d': (0, 0, 1, -1), 'e11': (1, 0, 0, 0), 'e22': (0, 0, 0, 1)}
ASLOT = {'I': 0, 'Z': 1, 'se1': 2, 'de1': 3, 'se2': 4, 'de2': 5, 'e1s': 6, 'e2s': 7,
         'e1d': 8, 'e2d': 10, 'e11': 12, 'e22': 14}
PLAN = [['I', 'se1', 'de1', 'e2s'], ['e1d', 'e11'], ['Z', 'se2', 'de2', 'e1s'], ['e2d', 'e22']]
PLAN0 = [['se1', 'de1', 'se2', 'de2'], ['e1d', 'e11'], ['I', 'Z', 'e1s', 'e2s'], ['e2d', 'e22']]
NPIECE = 20
STAT_STEPS = [2] * 16 + [1] * 4
BLOCKS = [[(0, 128)], [(128, 128)], [(256, 128)], [(384, 128)], [(512, 64), (544, 32), (512, 32)]]


def _dot(a, b):
    return jnp.dot(a, b, preferred_element_type=F32)


def _pk16(lo, hi):
    return pltpu.pack_elementwise([lo, hi], packed_dtype=BF16)


def _upk(v):
    return pltpu.bitcast(v, BF16)


def _bits(v):
    return pltpu.bitcast(v, U32)


def _link(v, zero):
    return pltpu.bitcast(_bits(v) | zero, F32)


def _lane_arrange(v_ref):
    v8 = jnp.broadcast_to(v_ref[...].astype(F32).reshape(1, D), (8, D))
    lane = jax.lax.broadcasted_iota(jnp.int32, (8, 128), 1)
    perm = (lane & ~15) | ((lane & 15) >> 1) | ((lane & 1) << 3)
    out = [jnp.take_along_axis(v8[:, 128 * i:128 * (i + 1)], perm, axis=1) for i in range(4)]
    last = jnp.concatenate([v8[:, 512:], v8[:, 512:]], axis=1)
    idx = jnp.where(lane < 64, perm, jnp.where(lane < 96, perm - 32, perm - 96))
    out.append(jnp.take_along_axis(last, idx, axis=1))
    return out


def _transpose_w(w_ref, wt_ref, blocks):
    for bi in blocks:
        for c in range(5):
            wd = min(128, D - 128 * c)
            rows = []
            for st, ln in BLOCKS[bi]:
                w = w_ref[st:st + ln, 128 * c:128 * c + wd].astype(F32).reshape(ln // 16, 16, wd)
                rows.append(_pk16(w[:, :8], w[:, 8:]).reshape(ln // 2, wd))
            wp = jnp.concatenate(rows, axis=0) if len(rows) > 1 else rows[0]
            wt_ref[bi, 64 * c:64 * c + wd // 2, :] = _bits(_upk(wp).T)


def _prep_a(gt, wt_ref, a_ref, slots):
    lane = jax.lax.broadcasted_iota(jnp.int32, (8, 128), 1)

    def s96(a, b):
        return jnp.where(lane < 96, a, b)

    def es(sv, sx, sy):
        return jnp.where(lane < 64, sv, s96(pltpu.roll(sx, 96, 1), sy))

    for j in range(NH // 16):
        res = []
        for par in range(2):
            memo = {}

            def n(h, bi):
                if (h, bi) not in memo:
                    r0 = 8 * (j + (h - 1) * (NH // 16))
                    memo[(h, bi)] = gt[bi] * pltpu.unpack_elementwise(
                        wt_ref[bi, r0:r0 + 8, :], index=par, packed_dtype=BF16, unpacked_dtype=F32)
                return memo[(h, bi)]

            def c(h1, b1, sg, h2, b2):
                key = (h1, b1, sg, h2, b2)
                if key not in memo:
                    memo[key] = n(h1, b1) + n(h2, b2) if sg > 0 else n(h1, b1) - n(h2, b2)
                return memo[key]

            fns = [
                lambda: s96(c(1, 0, 1, 2, 1), c(1, 2, -1, 2, 3)),
                lambda: s96(c(1, 2, -1, 2, 3), c(1, 0, 1, 2, 1)),
                lambda: n(2, 1), lambda: -n(2, 3), lambda: n(1, 0), lambda: n(1, 2),
                lambda: es(n(1, 4), c(1, 0, 1, 1, 1), c(1, 2, 1, 1, 3)),
                lambda: es(n(2, 4), c(2, 0, 1, 2, 1), c(2, 2, 1, 2, 3)),
                lambda: s96(-c(1, 0, 1, 1, 1), n(1, 4)),
                lambda: s96(-c(1, 2, 1, 1, 3), pltpu.roll(n(1, 4), 32, 1)),
                lambda: s96(c(2, 0, 1, 2, 1), n(2, 4)),
                lambda: s96(c(2, 2, 1, 2, 3), pltpu.roll(n(2, 4), 32, 1)),
                lambda: c(1, 1, -1, 2, 1), lambda: c(1, 3, 1, 2, 3),
                lambda: s96(c(2, 0, -1, 1, 0), -c(2, 0, -1, 1, 0)),
                lambda: s96(c(2, 2, 1, 1, 2), -c(2, 2, 1, 1, 2)),
            ]
            res.append([fns[i]() for i in slots])
        for i, ev, od in zip(slots, *res):
            a_ref[i, 8 * j:8 * j + 8, :] = _pk16(ev, od)


class _Stats:
    def __init__(self, x_view):
        self.x = x_view
        self.p0 = jnp.broadcast_to(x_view[0:G, :].astype(F32)[0:1], (8, W2))
        self.p = self.p0
        self.s = None
        self.q = None
        self.k = 0

    def step(self, n):
        for _ in range(n):
            x = self.x[self.k * G:(self.k + 1) * G, :].astype(F32)
            for h in range(2):
                d = x[8 * h:8 * h + 8] - self.p
                self.s = d if self.s is None else self.s + d
                self.q = d * d if self.q is None else self.q + d * d
            self.k += 1

    def finish(self):
        s = jnp.sum(self.s, axis=0, keepdims=True) * (1.0 / D)
        q = jnp.sum(self.q, axis=0, keepdims=True) * (1.0 / D)
        var = jnp.maximum(q - s * s, 0.0)
        return self.p0[0:1] + s, jax.lax.rsqrt(var + EPS)


def _prep_tile(x_view, p_ref, cur, nxt_view, tick, t0, t1):
    def zz_at(t):
        z = tick(t)
        return jnp.concatenate([z, z], axis=1)

    if cur is None:
        st = _Stats(x_view)
        tm = t0 + (t1 - t0) * (0.33 if nxt_view is not None else 0.5)
        for k in range(12):
            if tick is not None:
                st.p = _link(st.p0, zz_at(t0 + (tm - t0) * k / 12))
            st.step(3)
        cur = st.finish()
        t0 = tm
    m, r = [jnp.broadcast_to(v, (8, W2)) for v in cur]
    st = None if nxt_view is None else _Stats(nxt_view)

    def add(a, b):
        return a[0] + b[0], a[1] + b[1]

    def sub(a, b):
        return a[0] - b[0], a[1] - b[1]

    for k in range(NPIECE):
        mm = m
        if tick is not None:
            zz = zz_at(t0 + (t1 - t0) * k / NPIECE)
            mm = _link(m, zz)
            if st is not None:
                st.p = _link(st.p0, zz)

        def nrm(r0, mm=mm):
            x = x_view[r0:r0 + G, :].astype(F32)
            lo = (x[:8] - mm) * r
            hi = (x[8:] - mm) * r
            return (lo[:, :T], hi[:, :T]), (lo[:, T:], hi[:, T:])

        if st is not None:
            st.step(STAT_STEPS[k])
        if k < 16:
            r0 = (k // 8) * 256 + (k % 8) * G
            b11, b12 = nrm(r0)
            b21, b22 = nrm(r0 + 128)
            pm = add if k % 8 < 6 else sub
            vals = [pm(b11, b22), b11, sub(b12, b22), sub(b21, b11), b22, pm(b11, b12), pm(b21, b22)]
            for i, v in enumerate(vals):
                q0 = i * 128 + k * 8
                p_ref[q0:q0 + 8, :] = _pk16(*v)
        else:
            kk = k - 16
            b1, b2 = nrm(512 + kk * G)
            p_ref[SP + kk * 8:SP + kk * 8 + 8, :] = _pk16(*add(b1, b2))
            p_ref[SM + kk * 8:SM + kk * 8 + 8, :] = _pk16(*sub(b1, b2))
    return None if st is None else st.finish()


def _mm_tile(p_ref, a_ref, bias_ref, obuf, s, cols, plan, stored):
    m = {}
    acc = [None] * 4
    for rnd in plan:
        for nm in rnd:
            parts = [p_ref[q0:q0 + n, :] for q0, n in PASSES[nm]]
            rhs = _upk(jnp.concatenate(parts, axis=0) if len(parts) > 1 else parts[0])
            sl = ASLOT[nm]
            lhs = a_ref[sl] if rhs.shape[0] == 128 else jnp.concatenate([a_ref[sl], a_ref[sl + 1]], axis=1)
            m[nm] = _dot(_upk(lhs), rhs)
        for q in range(4):
            terms = [(nm, SIGMA[nm][q]) for nm in rnd if SIGMA[nm][q]]
            if not terms:
                continue
            s0 = terms[0][1]
            val = m[terms[0][0]]
            for nm, sg in terms[1:]:
                val = val + m[nm] if sg * s0 > 0 else val - m[nm]
            prev = acc[q] if acc[q] is not None else (bias_ref[:NH, :] if q < 2 else bias_ref[NH:, :])
            acc[q] = prev + val if s0 > 0 else prev - val
    for h in range(2):
        obuf[2 * s + h, :, cols] = jnp.concatenate(acc[2 * h:2 * h + 2], axis=1).astype(BF16)
        if stored is not None:
            stored(h)
    return m


def _write_runs(groups, nhead, tpi, tau_w, lead):
    runs = {}
    h0 = 0
    for n in groups:
        tau = max(tau_w + max(h0 - lead, 0), 2 * (h0 + n))
        i, u = divmod(tau - nhead, tpi)
        lst = runs.setdefault(u, [])
        prev = lst[-1] if lst else None
        if prev and prev[1] == i - 1 and prev[4] == n and prev[3] in (None, (h0 - prev[2]) / (i - prev[0])):
            lst[-1] = (prev[0], i, prev[2], (h0 - prev[2]) // (i - prev[0]), n)
        else:
            lst.append((i, i, h0, None, n))
        h0 += n
    return runs


def _body(x_hbm, g_hbm, b_hbm, w_hbm, o_hbm, xbuf, obuf, wbuf, gbuf, bbuf, wt_ref, a_ref, bias_ref,
          pa, pb, z_ref, isem, osem, *, U, head, groups, tau_w, lead, spans, b0):
    S, _, B = x_hbm.shape
    NT = B // W2
    nhead = sum(head)
    hs = nhead // NT
    NIT = (S - hs) // U
    TPI = U * NT
    pbuf = (pa, pb)

    def rd_cols(s, t0, n, k):
        return pltpu.make_async_copy(
            x_hbm.at[s, :, pl.ds(t0 * W2, n * W2)], xbuf.at[s, :, pl.ds(t0 * W2, n * W2)], isem.at[k])

    def rd(s0, n, k):
        return pltpu.make_async_copy(x_hbm.at[pl.ds(s0, n)], xbuf.at[pl.ds(s0, n)], isem.at[k])

    def wr(h0, n, segs):
        for j in segs:
            idx = (pl.ds(h0, n), pl.ds(j * SEG, SEG))
            pltpu.make_async_copy(obuf.at[idx], o_hbm.at[idx], osem.at[0]).start()

    def wr_cols(h0, n, cols):
        idx = (pl.ds(h0, n), slice(None), cols)
        pltpu.make_async_copy(obuf.at[idx], o_hbm.at[idx], osem.at[0]).start()

    def tile(s, t):
        return xbuf.at[s, :, pl.ds(t * W2, W2)]

    first = [pltpu.make_async_copy(g_hbm, gbuf, isem.at[0]),
             pltpu.make_async_copy(b_hbm, bbuf, isem.at[0]),
             pltpu.make_async_copy(w_hbm, wbuf, isem.at[0])]
    x0 = rd_cols(0, 0, 1, 1)
    have = 1
    head_waits = []
    pos = 0
    for bi, n in enumerate(head):
        need = pos + n + (1 if bi == 0 else 2)
        if bi == len(head) - 1 or need > 2 * NT:
            need = -(-need // NT) * NT
        cps = []
        while have < need:
            s, t = divmod(have, NT)
            if t == 0 and need - have >= NT:
                ns = (need - have) // NT
                cps.append(rd(s, ns, 2 + bi))
                have += ns * NT
            else:
                nt = min(NT - t, need - have)
                cps.append(rd_cols(s, t, nt, 2 + bi))
                have += nt
        head_waits.append(cps)
        pos += n
    k0 = 2 + len(head)

    def loop_rd(i):
        return rd(hs + 1 + U * i, U, k0 + i)

    last_rd = rd(S - U + 1, U - 1, k0 + NIT - 1)
    for cp in (first + [x0] + [c for cs in head_waits for c in cs]
               + [loop_rd(i) for i in range(NIT - 1)] + [last_rd]):
        cp.start()

    for cp in first:
        cp.wait()
    _transpose_w(wbuf, wt_ref, range(5))
    brow = _dot(jnp.broadcast_to(bbuf[...].reshape(1, D), (16, D)), wbuf[...])[0:1]
    x0.wait()
    bias_ref[...] = jnp.broadcast_to(brow, (T, D)).T
    z_ref[...] = jnp.zeros(z_ref.shape, U32)
    gt = _lane_arrange(gbuf)
    gt[4] = gt[4] * 0.5
    _prep_tile(tile(0, 0), pa, None, None, None, 0, 0)
    early = [2, 3, 4, 5]
    _prep_a(gt, wt_ref, a_ref, early)

    def block(st, s0, t0, n, stored=None, first=False):
        z = z_ref[...]
        for u in range(n):
            tt = t0 + u
            ds, t = divmod(tt, NT)

            def view(q):
                d2, t2 = divmod(q, NT)
                s2 = s0 + d2
                if not isinstance(s2, int) and d2 == U:
                    s2 = jnp.minimum(s2, S - 1)
                return tile(s2, t2)

            plan = PLAN0 if first else PLAN
            m = _mm_tile(pbuf[tt % 2], a_ref, bias_ref, obuf, s0 + ds, pl.ds(t * W2, W2), plan,
                         stored and functools.partial(stored, tt))

            def tick(tm, m=m, plan=plan):
                return _bits(m[plan[int(tm // NH)][0]][int(tm % NH) // 8 * 8:][:8]) & z

            st = _prep_tile(view(tt + 1), pbuf[(tt + 1) % 2], st, None if first else view(tt + 2), tick,
                            b0 if first else 0, spans[0] if u < n - 1 else spans[1])
        return st

    pos = 0
    st = None
    for bi, (n, cps) in enumerate(zip(head, head_waits)):
        for cp in cps:
            cp.wait()
        if bi == 0:
            _prep_a(gt, wt_ref, a_ref, [i for i in range(16) if i not in early])
        st = block(st, 0, pos, n, first=bi == 0)
        pos += n

    runs = _write_runs(groups, nhead, TPI, tau_w, lead)

    def it(i, st):
        last = i == NIT - 1

        @pl.when(jnp.logical_not(last))
        def _():
            loop_rd(i).wait()

        @pl.when(last)
        def _():
            last_rd.wait()

        def issue(u, part):
            half = NH // SEG // 2
            for i0, i1, hh, dh, n in runs.get(u, []):
                @pl.when(jnp.logical_and(i >= i0, i <= i1))
                def _():
                    wr(hh if dh is None else hh + dh * (i - i0), n, range(part * half, (part + 1) * half))

        def stored(tt, h):
            if h == 0:
                issue(tt, 1)
            elif tt + 1 < TPI:
                issue(tt + 1, 0)
            if tt // NT == U - 1 and (h == 1 or tt == TPI - 1):
                @pl.when(last)
                def _():
                    cols = pl.ds((tt % NT) * W2, W2)
                    if tt == TPI - 1:
                        wr_cols(2 * (S - 1) + h, 1, cols)
                    else:
                        wr_cols(2 * (S - 1), 2, cols)

        issue(0, 0)
        return block(st, hs + i * U, 0, TPI, stored)

    jax.lax.fori_loop(0, NIT, it, st)
    pltpu.make_async_copy(obuf, o_hbm, osem.at[0]).wait()


def _run(x, g, b, w, U=4, head=(1, 1, 2, 4, 8), groups=(8,) * 7 + (4, 2), tau_w=62, lead=4,
         spans=(930, 1050), b0=250):
    B, S, _ = x.shape
    xt = jnp.transpose(x, (1, 2, 0))
    oshape = (2 * S, NH, B)
    nsem = 2 + len(head) + (S - sum(head) * W2 // B) // U
    out = pl.pallas_call(
        functools.partial(_body, U=U, head=head, groups=groups, tau_w=tau_w, lead=lead, spans=spans, b0=b0),
        in_specs=[pl.BlockSpec(memory_space=pl.ANY)] * 4,
        out_specs=pl.BlockSpec(memory_space=pl.ANY),
        out_shape=jax.ShapeDtypeStruct(oshape, x.dtype),
        scratch_shapes=[
            pltpu.VMEM((S, D, B), BF16),
            pltpu.VMEM(oshape, BF16),
            pltpu.VMEM((D, D), BF16),
            pltpu.VMEM((D,), BF16),
            pltpu.VMEM((D,), BF16),
            pltpu.VMEM((5, D // 2, 128), U32),
            pltpu.VMEM((16, NH // 2, 128), U32),
            pltpu.VMEM((D, T), F32),
            pltpu.VMEM((PROWS, T), U32),
            pltpu.VMEM((PROWS, T), U32),
            pltpu.VMEM((8, T), U32),
            pltpu.SemaphoreType.DMA((nsem,)),
            pltpu.SemaphoreType.DMA((1,)),
        ],
        compiler_params=pltpu.CompilerParams(
            vmem_limit_bytes=110 * 1024 * 1024,
            disable_bounds_checks=True,
            disable_semaphore_checks=True,
        ),
    )(xt, g, b, w)
    return jnp.transpose(out.reshape(S, D, B), (2, 0, 1))


@jax.jit
def pallas_standalone__layernorm_linear__sampling_kernel(x, g, b, w):
    return _run(x, g, b, w)
```

```python
import functools

import jax
import jax.numpy as jnp
import jax.experimental.pallas as pl
import jax.experimental.pallas.tpu as pltpu

EPS = 1e-5
F32 = jnp.float32
BF16 = jnp.bfloat16
U32 = jnp.uint32

D = 576
G = 16
T = 128
W2 = 2 * T
NH = D // 2
SEG = 16
PROWS = 7 * 128 + 64
SP, SM = 7 * 128, 7 * 128 + 32


def _rows(i, lo, hi):
    return (i - 1) * 128 + lo // 2, (hi - lo) // 2


PASSES = {
    'I': [_rows(1, 0, 96), _rows(1, 224, 256)],
    'Z': [_rows(1, 128, 224), _rows(1, 96, 128)],
    'se1': [_rows(4, 0, 128)], 'de1': [_rows(4, 128, 256)],
    'se2': [_rows(3, 0, 128)], 'de2': [_rows(3, 128, 256)],
    'e1s': [(SP, 32), _rows(5, 96, 128), _rows(5, 224, 256)],
    'e2s': [(SP, 32), _rows(2, 96, 128), _rows(2, 224, 256)],
    'e1d': [_rows(5, 0, 96), (SM, 16), _rows(5, 128, 224), (SM + 16, 16)],
    'e2d': [_rows(2, 0, 96), (SM, 16), _rows(2, 128, 224), (SM + 16, 16)],
    'e11': [_rows(7, 0, 256)], 'e22': [_rows(6, 0, 256)],
}
SIGMA = {'I': (1, 0, 0, 1), 'Z': (1, 0, 0, -1), 'se1': (1, 0, 1, 0), 'de1': (1, 0, -1, 0),
         'se2': (0, 1, 0, 1), 'de2': (0, 1, 0, -1), 'e1s': (1, 1, 0, 0), 'e1d': (1, -1, 0, 0),
         'e2s': (0, 0, 1, 1), 'e2d': (0, 0, 1, -1), 'e11': (1, 0, 0, 0), 'e22': (0, 0, 0, 1)}
ASLOT = {'I': 0, 'Z': 1, 'se1': 2, 'de1': 3, 'se2': 4, 'de2': 5, 'e1s': 6, 'e2s': 7,
         'e1d': 8, 'e2d': 10, 'e11': 12, 'e22': 14}
PLAN = [['I', 'se1', 'de1', 'e2s'], ['e1d', 'e11'], ['Z', 'se2', 'de2', 'e1s'], ['e2d', 'e22']]
NPIECE = 20
STAT_STEPS = [2] * 16 + [1] * 4
W_STEPS = [([4, 1, 3], []), ([0, 2], [2, 3, 12, 13])]
BLOCKS = [[(0, 128)], [(128, 128)], [(256, 128)], [(384, 128)], [(512, 64), (544, 32), (512, 32)]]


def _dot(a, b):
    return jnp.dot(a, b, preferred_element_type=F32)


def _pk16(lo, hi):
    return pltpu.pack_elementwise([lo, hi], packed_dtype=BF16)


def _upk(v):
    return pltpu.bitcast(v, BF16)


def _bits(v):
    return pltpu.bitcast(v, U32)


def _link(v, zero):
    return pltpu.bitcast(_bits(v) | zero, F32)


def _lane_arrange(v_ref):
    v8 = jnp.broadcast_to(v_ref[...].astype(F32).reshape(1, D), (8, D))
    lane = jax.lax.broadcasted_iota(jnp.int32, (8, 128), 1)
    perm = (lane & ~15) | ((lane & 15) >> 1) | ((lane & 1) << 3)
    out = [jnp.take_along_axis(v8[:, 128 * i:128 * (i + 1)], perm, axis=1) for i in range(4)]
    last = jnp.concatenate([v8[:, 512:], v8[:, 512:]], axis=1)
    idx = jnp.where(lane < 64, perm, jnp.where(lane < 96, perm - 32, perm - 96))
    out.append(jnp.take_along_axis(last, idx, axis=1))
    return out


def _transpose_w(w_ref, wt_ref, blocks):
    for bi in blocks:
        for c in range(5):
            wd = min(128, D - 128 * c)
            rows = []
            for st, ln in BLOCKS[bi]:
                w = w_ref[st:st + ln, 128 * c:128 * c + wd].astype(F32).reshape(ln // 16, 16, wd)
                rows.append(_pk16(w[:, :8], w[:, 8:]).reshape(ln // 2, wd))
            wp = jnp.concatenate(rows, axis=0) if len(rows) > 1 else rows[0]
            wt_ref[bi, 64 * c:64 * c + wd // 2, :] = _bits(_upk(wp).T)


def _prep_a(gt, wt_ref, a_ref, slots):
    lane = jax.lax.broadcasted_iota(jnp.int32, (8, 128), 1)

    def s96(a, b):
        return jnp.where(lane < 96, a, b)

    def es(sv, sx, sy):
        return jnp.where(lane < 64, sv, s96(pltpu.roll(sx, 96, 1), sy))

    for j in range(NH // 16):
        res = []
        for par in range(2):
            memo = {}

            def n(h, bi):
                if (h, bi) not in memo:
                    r0 = 8 * (j + (h - 1) * (NH // 16))
                    memo[(h, bi)] = gt[bi] * pltpu.unpack_elementwise(
                        wt_ref[bi, r0:r0 + 8, :], index=par, packed_dtype=BF16, unpacked_dtype=F32)
                return memo[(h, bi)]

            def c(h1, b1, sg, h2, b2):
                key = (h1, b1, sg, h2, b2)
                if key not in memo:
                    memo[key] = n(h1, b1) + n(h2, b2) if sg > 0 else n(h1, b1) - n(h2, b2)
                return memo[key]

            fns = [
                lambda: s96(c(1, 0, 1, 2, 1), c(1, 2, -1, 2, 3)),
                lambda: s96(c(1, 2, -1, 2, 3), c(1, 0, 1, 2, 1)),
                lambda: n(2, 1), lambda: -n(2, 3), lambda: n(1, 0), lambda: n(1, 2),
                lambda: es(n(1, 4), c(1, 0, 1, 1, 1), c(1, 2, 1, 1, 3)),
                lambda: es(n(2, 4), c(2, 0, 1, 2, 1), c(2, 2, 1, 2, 3)),
                lambda: s96(-c(1, 0, 1, 1, 1), n(1, 4)),
                lambda: s96(-c(1, 2, 1, 1, 3), pltpu.roll(n(1, 4), 32, 1)),
                lambda: s96(c(2, 0, 1, 2, 1), n(2, 4)),
                lambda: s96(c(2, 2, 1, 2, 3), pltpu.roll(n(2, 4), 32, 1)),
                lambda: c(1, 1, -1, 2, 1), lambda: c(1, 3, 1, 2, 3),
                lambda: s96(c(2, 0, -1, 1, 0), -c(2, 0, -1, 1, 0)),
                lambda: s96(c(2, 2, 1, 1, 2), -c(2, 2, 1, 1, 2)),
            ]
            res.append([fns[i]() for i in slots])
        for i, ev, od in zip(slots, *res):
            a_ref[i, 8 * j:8 * j + 8, :] = _pk16(ev, od)


class _Stats:
    def __init__(self, x_view):
        self.x = x_view
        self.p0 = jnp.broadcast_to(x_view[0:G, :].astype(F32)[0:1], (8, W2))
        self.p = self.p0
        self.s = None
        self.q = None
        self.k = 0

    def step(self, n):
        for _ in range(n):
            x = self.x[self.k * G:(self.k + 1) * G, :].astype(F32)
            for h in range(2):
                d = x[8 * h:8 * h + 8] - self.p
                self.s = d if self.s is None else self.s + d
                self.q = d * d if self.q is None else self.q + d * d
            self.k += 1

    def finish(self):
        s = jnp.sum(self.s, axis=0, keepdims=True) * (1.0 / D)
        q = jnp.sum(self.q, axis=0, keepdims=True) * (1.0 / D)
        var = jnp.maximum(q - s * s, 0.0)
        return self.p0[0:1] + s, jax.lax.rsqrt(var + EPS)


def _prep_tile(x_view, p_ref, cur, nxt_view, tick, t0, t1):
    def zz_at(t):
        z = tick(t)
        return jnp.concatenate([z, z], axis=1)

    if cur is None:
        st = _Stats(x_view)
        tm = t0 + (t1 - t0) * (0.33 if nxt_view is not None else 0.5)
        for k in range(12):
            if tick is not None:
                st.p = _link(st.p0, zz_at(t0 + (tm - t0) * k / 12))
            st.step(3)
        cur = st.finish()
        t0 = tm
    m, r = [jnp.broadcast_to(v, (8, W2)) for v in cur]
    st = None if nxt_view is None else _Stats(nxt_view)

    def add(a, b):
        return a[0] + b[0], a[1] + b[1]

    def sub(a, b):
        return a[0] - b[0], a[1] - b[1]

    for k in range(NPIECE):
        mm = m
        if tick is not None:
            zz = zz_at(t0 + (t1 - t0) * k / NPIECE)
            mm = _link(m, zz)
            if st is not None:
                st.p = _link(st.p0, zz)

        def nrm(r0, mm=mm):
            x = x_view[r0:r0 + G, :].astype(F32)
            lo = (x[:8] - mm) * r
            hi = (x[8:] - mm) * r
            return (lo[:, :T], hi[:, :T]), (lo[:, T:], hi[:, T:])

        if st is not None:
            st.step(STAT_STEPS[k])
        if k < 16:
            r0 = (k // 8) * 256 + (k % 8) * G
            b11, b12 = nrm(r0)
            b21, b22 = nrm(r0 + 128)
            pm = add if k % 8 < 6 else sub
            vals = [pm(b11, b22), b11, sub(b12, b22), sub(b21, b11), b22, pm(b11, b12), pm(b21, b22)]
            for i, v in enumerate(vals):
                q0 = i * 128 + k * 8
                p_ref[q0:q0 + 8, :] = _pk16(*v)
        else:
            kk = k - 16
            b1, b2 = nrm(512 + kk * G)
            p_ref[SP + kk * 8:SP + kk * 8 + 8, :] = _pk16(*add(b1, b2))
            p_ref[SM + kk * 8:SM + kk * 8 + 8, :] = _pk16(*sub(b1, b2))
    return None if st is None else st.finish()


def _mm_tile(p_ref, a_ref, bias_ref, obuf, s, cols, plan, stored, bias_last=False):
    m = {}
    acc = [None] * 4
    for rnd in plan:
        for nm in rnd:
            parts = [p_ref[q0:q0 + n, :] for q0, n in PASSES[nm]]
            rhs = _upk(jnp.concatenate(parts, axis=0) if len(parts) > 1 else parts[0])
            sl = ASLOT[nm]
            lhs = a_ref[sl] if rhs.shape[0] == 128 else jnp.concatenate([a_ref[sl], a_ref[sl + 1]], axis=1)
            m[nm] = _dot(_upk(lhs), rhs)
        for q in range(4):
            terms = [(nm, SIGMA[nm][q]) for nm in rnd if SIGMA[nm][q]]
            if not terms:
                continue
            s0 = terms[0][1]
            val = m[terms[0][0]]
            for nm, sg in terms[1:]:
                val = val + m[nm] if sg * s0 > 0 else val - m[nm]
            if acc[q] is None and bias_last:
                acc[q] = val if s0 > 0 else -val
                continue
            prev = acc[q] if acc[q] is not None else (bias_ref[:NH, :] if q < 2 else bias_ref[NH:, :])
            acc[q] = prev + val if s0 > 0 else prev - val
    if bias_last:
        acc = [acc[q] + (bias_ref[:NH, :] if q < 2 else bias_ref[NH:, :]) for q in range(4)]
    for h in range(2):
        obuf[2 * s + h, :, cols] = jnp.concatenate(acc[2 * h:2 * h + 2], axis=1).astype(BF16)
        if stored is not None:
            stored(h)
    return m


def _write_runs(groups, nhead, tpi, tau_w, lead):
    runs = {}
    h0 = 0
    for n in groups:
        tau = max(tau_w + max(h0 - lead, 0), 2 * (h0 + n))
        i, u = divmod(tau - nhead, tpi)
        lst = runs.setdefault(u, [])
        prev = lst[-1] if lst else None
        if prev and prev[1] == i - 1 and prev[4] == n and prev[3] in (None, (h0 - prev[2]) / (i - prev[0])):
            lst[-1] = (prev[0], i, prev[2], (h0 - prev[2]) // (i - prev[0]), n)
        else:
            lst.append((i, i, h0, None, n))
        h0 += n
    return runs


def _body(x_hbm, g_hbm, b_hbm, w_hbm, o_hbm, xbuf, obuf, wbuf, gbuf, bbuf, wt_ref, a_ref, bias_ref,
          pa, pb, z_ref, isem, osem, *, U, head, groups, tau_w, lead, spans, strips):
    S, _, B = x_hbm.shape
    NT = B // W2
    nhead = sum(head)
    hs = nhead // NT
    NIT = (S - hs) // U
    TPI = U * NT
    pbuf = (pa, pb)

    def rd_cols(s, t0, n, k):
        return pltpu.make_async_copy(
            x_hbm.at[s, :, pl.ds(t0 * W2, n * W2)], xbuf.at[s, :, pl.ds(t0 * W2, n * W2)], isem.at[k])

    def rd(s0, n, k):
        return pltpu.make_async_copy(x_hbm.at[pl.ds(s0, n)], xbuf.at[pl.ds(s0, n)], isem.at[k])

    def wr(h0, n, segs):
        for j in segs:
            idx = (pl.ds(h0, n), pl.ds(j * SEG, SEG))
            pltpu.make_async_copy(obuf.at[idx], o_hbm.at[idx], osem.at[0]).start()

    def wr_cols(h0, n, cols):
        idx = (pl.ds(h0, n), slice(None), cols)
        pltpu.make_async_copy(obuf.at[idx], o_hbm.at[idx], osem.at[0]).start()

    def tile(s, t):
        return xbuf.at[s, :, pl.ds(t * W2, W2)]

    def rd_w(bi, k):
        rows = pl.ds(128 * bi, min(128, D - 128 * bi))
        return pltpu.make_async_copy(w_hbm.at[rows], wbuf.at[rows], isem.at[k])

    first = [pltpu.make_async_copy(g_hbm, gbuf, isem.at[0]), pltpu.make_async_copy(b_hbm, bbuf, isem.at[0])]
    w_rd = [[rd_w(bi, k) for bi in bis] for k, (bis, _) in enumerate(W_STEPS)]
    kx = len(W_STEPS)
    x0 = rd_cols(0, 0, 1, kx)

    def rd_tiles(lo, hi, k):
        cps = []
        while lo < hi:
            s, t = divmod(lo, NT)
            n = (hi - lo) // NT * NT if t == 0 and hi - lo >= NT else min(NT - t, hi - lo)
            cps.append(rd(s, n // NT, k) if t == 0 and n >= NT else rd_cols(s, t, n, k))
            lo += n
        return cps

    ends = [2] + [sum(head[:bi + 1]) + 2 for bi in range(1, len(head))]
    ends += [min(nhead + TPI * (i + 1) + 2, S * NT) for i in range(NIT)]
    chunks = [rd_tiles(lo, hi, kx + 1 + k) for k, (lo, hi) in enumerate(zip([1] + ends, ends))]
    head_waits = chunks[:len(head)]
    k0 = kx + 1 + len(head)
    for cp in first + sum(w_rd, []) + [x0] + sum(chunks, []):
        cp.start()

    for cp in first:
        cp.wait()
    gt = None
    for cps, (bis, slots) in zip(w_rd, W_STEPS):
        for cp in cps:
            cp.wait()
        _transpose_w(wbuf, wt_ref, bis)
        if gt is None:
            gt = _lane_arrange(gbuf)
            gt[4] = gt[4] * 0.5
        _prep_a(gt, wt_ref, a_ref, slots)
    brow = _dot(jnp.broadcast_to(bbuf[...].reshape(1, D), (16, D)), wbuf[...])[0:1]
    x0.wait()
    z_ref[...] = jnp.zeros(z_ref.shape, U32)
    _prep_tile(tile(0, 0), pa, None, None, None, 0, 0)
    _prep_a(gt, wt_ref, a_ref, [i for i in range(16) if not any(i in sl for _, sl in W_STEPS)])

    def block(st, s0, t0, n, stored=None, first=False):
        z = z_ref[...]
        for u in range(n):
            tt = t0 + u
            ds, t = divmod(tt, NT)

            def view(q):
                d2, t2 = divmod(q, NT)
                s2 = s0 + d2
                if not isinstance(s2, int) and d2 == U:
                    s2 = jnp.minimum(s2, S - 1)
                return tile(s2, t2)

            m = _mm_tile(pbuf[tt % 2], a_ref, bias_ref, obuf, s0 + ds, pl.ds(t * W2, W2), PLAN,
                         stored and functools.partial(stored, tt), first)

            def tick(tm, m=m):
                return _bits(m[PLAN[int(tm // NH)][0]][int(tm % NH) // 8 * 8:][:8]) & z

            st = _prep_tile(view(tt + 1), pbuf[(tt + 1) % 2], st, None if first else view(tt + 2), tick,
                            0, spans[0] if u < n - 1 else spans[1])
        return st

    pos = 0
    st = None
    for bi, (n, cps) in enumerate(zip(head, head_waits)):
        for cp in cps:
            cp.wait()
        if bi == 0:
            bias_ref[...] = jnp.broadcast_to(brow, (T, D)).T
        st = block(st, 0, pos, n, first=bi == 0)
        pos += n

    runs = _write_runs(groups, nhead, TPI, tau_w, lead)

    def it(i, st):
        last = i == NIT - 1

        @pl.when(jnp.logical_not(last))
        def _():
            rd(0, U, k0 + i).wait()

        @pl.when(last)
        def _():
            for cp in chunks[-1]:
                cp.wait()

        def issue(u, part):
            half = NH // SEG // 2
            for i0, i1, hh, dh, n in runs.get(u, []):
                @pl.when(jnp.logical_and(i >= i0, i <= i1))
                def _():
                    wr(hh if dh is None else hh + dh * (i - i0), n, range(part * half, (part + 1) * half))

        def stored(tt, h):
            if h == 0:
                issue(tt, 1)
            elif tt + 1 < TPI:
                issue(tt + 1, 0)
            back = TPI - 1 - tt
            strip = strips[back] if back < len(strips) else 0
            if strip and (h == 1 or back == 0):
                @pl.when(last)
                def _():
                    h0 = 2 * (S - 1 - back // NT)
                    cols = pl.ds((tt % NT + 1 - strip) * W2, strip * W2)
                    if back == 0:
                        wr_cols(h0 + h, 1, cols)
                    else:
                        wr_cols(h0, 2, cols)

        issue(0, 0)
        return block(st, hs + i * U, 0, TPI, stored)

    jax.lax.fori_loop(0, NIT, it, st)
    pltpu.make_async_copy(obuf, o_hbm, osem.at[0]).wait()


def _run(x, g, b, w, U=4, head=(1, 1, 2, 4, 8), groups=(8,) * 6 + (4, 4, 2, 2), tau_w=62, lead=4,
         spans=(930, 1050), strips=(1, 1, 1, 1, 2, 0, 2)):
    B, S, _ = x.shape
    xt = jnp.transpose(x, (1, 2, 0))
    oshape = (2 * S, NH, B)
    nsem = len(W_STEPS) + 1 + len(head) + (S - sum(head) * W2 // B) // U
    out = pl.pallas_call(
        functools.partial(_body, U=U, head=head, groups=groups, tau_w=tau_w, lead=lead, spans=spans,
                          strips=strips),
        in_specs=[pl.BlockSpec(memory_space=pl.ANY)] * 4,
        out_specs=pl.BlockSpec(memory_space=pl.ANY),
        out_shape=jax.ShapeDtypeStruct(oshape, x.dtype),
        scratch_shapes=[
            pltpu.VMEM((S, D, B), BF16),
            pltpu.VMEM(oshape, BF16),
            pltpu.VMEM((D, D), BF16),
            pltpu.VMEM((D,), BF16),
            pltpu.VMEM((D,), BF16),
            pltpu.VMEM((5, D // 2, 128), U32),
            pltpu.VMEM((16, NH // 2, 128), U32),
            pltpu.VMEM((D, T), F32),
            pltpu.VMEM((PROWS, T), U32),
            pltpu.VMEM((PROWS, T), U32),
            pltpu.VMEM((8, T), U32),
            pltpu.SemaphoreType.DMA((nsem,)),
            pltpu.SemaphoreType.DMA((1,)),
        ],
        compiler_params=pltpu.CompilerParams(
            vmem_limit_bytes=110 * 1024 * 1024,
            disable_bounds_checks=True,
            disable_semaphore_checks=True,
        ),
    )(xt, g, b, w)
    return jnp.transpose(out.reshape(S, D, B), (2, 0, 1))


@jax.jit
def pallas_standalone__layernorm_linear__sampling_kernel(x, g, b, w):
    return _run(x, g, b, w)
```

```python
import functools

import jax
import jax.numpy as jnp
import jax.experimental.pallas as pl
import jax.experimental.pallas.tpu as pltpu

EPS = 1e-5
F32 = jnp.float32
BF16 = jnp.bfloat16
U32 = jnp.uint32

D = 576
G = 16
T = 128
W2 = 2 * T
NH = D // 2
SEG = 16
PROWS = 7 * 256 + 128
SP, SM = 7 * 256, 7 * 256 + 64


def _rows(i, lo, hi):
    return (i - 1) * 256 + lo, hi - lo


PASSES = {
    'I': [_rows(1, 0, 96), _rows(1, 224, 256)],
    'Z': [_rows(1, 128, 224), _rows(1, 96, 128)],
    'se1': [_rows(4, 0, 128)], 'de1': [_rows(4, 128, 256)],
    'se2': [_rows(3, 0, 128)], 'de2': [_rows(3, 128, 256)],
    'e1s': [(SP, 64), _rows(5, 96, 128), _rows(5, 224, 256)],
    'e2s': [(SP, 64), _rows(2, 96, 128), _rows(2, 224, 256)],
    'e1d': [_rows(5, 0, 96), (SM, 32), _rows(5, 128, 224), (SM + 32, 32)],
    'e2d': [_rows(2, 0, 96), (SM, 32), _rows(2, 128, 224), (SM + 32, 32)],
    'e11': [_rows(7, 0, 256)], 'e22': [_rows(6, 0, 256)],
}
SIGMA = {'I': (1, 0, 0, 1), 'Z': (1, 0, 0, -1), 'se1': (1, 0, 1, 0), 'de1': (1, 0, -1, 0),
         'se2': (0, 1, 0, 1), 'de2': (0, 1, 0, -1), 'e1s': (1, 1, 0, 0), 'e1d': (1, -1, 0, 0),
         'e2s': (0, 0, 1, 1), 'e2d': (0, 0, 1, -1), 'e11': (1, 0, 0, 0), 'e22': (0, 0, 0, 1)}
ASLOT = {'I': 0, 'Z': 1, 'se1': 2, 'de1': 3, 'se2': 4, 'de2': 5, 'e1s': 6, 'e2s': 7,
         'e1d': 8, 'e2d': 10, 'e11': 12, 'e22': 14}
PLAN = [['I', 'se1', 'de1', 'e2s'], ['e1d', 'e11'], ['Z', 'se2', 'de2', 'e1s'], ['e2d', 'e22']]
NPIECE = 20
STAT_STEPS = [2] * 16 + [1] * 4
W_STEPS = [([4, 1, 3], []), ([0, 2], [2, 3, 12, 13])]
BLOCKS = [[(0, 128)], [(128, 128)], [(256, 128)], [(384, 128)], [(512, 64), (544, 32), (512, 32)]]


def _dot(a, b):
    return jnp.dot(a, b, preferred_element_type=F32)


def _upk(v):
    return pltpu.bitcast(v, BF16)


def _bits(v):
    return pltpu.bitcast(v, U32)


def _link(v, zero):
    return pltpu.bitcast(_bits(v) | zero, F32)


def _transpose_w(w_ref, wt_ref, blocks):
    for bi in blocks:
        for c in range(5):
            wd = min(128, D - 128 * c)
            rows = [w_ref[st:st + ln, 128 * c:128 * c + wd] for st, ln in BLOCKS[bi]]
            wp = jnp.concatenate(rows, axis=0) if len(rows) > 1 else rows[0]
            wt_ref[bi, 64 * c:64 * c + wd // 2, :] = _bits(wp.T)


def _prep_a(gt, wt_ref, a_ref, slots):
    lane = jax.lax.broadcasted_iota(jnp.int32, (G, 128), 1)

    def s96(a, b):
        return jnp.where(lane < 96, a, b)

    def es(sv, sx, sy):
        return jnp.where(lane < 64, sv, s96(pltpu.roll(sx, 96, 1), sy))

    for j in range(NH // G):
        memo = {}

        def n(h, bi):
            if (h, bi) not in memo:
                r0 = 8 * (j + (h - 1) * (NH // G))
                memo[(h, bi)] = gt[bi] * _upk(wt_ref[bi, r0:r0 + 8, :]).astype(F32)
            return memo[(h, bi)]

        def c(h1, b1, sg, h2, b2):
            key = (h1, b1, sg, h2, b2)
            if key not in memo:
                memo[key] = n(h1, b1) + n(h2, b2) if sg > 0 else n(h1, b1) - n(h2, b2)
            return memo[key]

        fns = [
            lambda: s96(c(1, 0, 1, 2, 1), c(1, 2, -1, 2, 3)),
            lambda: s96(c(1, 2, -1, 2, 3), c(1, 0, 1, 2, 1)),
            lambda: n(2, 1), lambda: -n(2, 3), lambda: n(1, 0), lambda: n(1, 2),
            lambda: es(n(1, 4), c(1, 0, 1, 1, 1), c(1, 2, 1, 1, 3)),
            lambda: es(n(2, 4), c(2, 0, 1, 2, 1), c(2, 2, 1, 2, 3)),
            lambda: s96(-c(1, 0, 1, 1, 1), n(1, 4)),
            lambda: s96(-c(1, 2, 1, 1, 3), pltpu.roll(n(1, 4), 32, 1)),
            lambda: s96(c(2, 0, 1, 2, 1), n(2, 4)),
            lambda: s96(c(2, 2, 1, 2, 3), pltpu.roll(n(2, 4), 32, 1)),
            lambda: c(1, 1, -1, 2, 1), lambda: c(1, 3, 1, 2, 3),
            lambda: s96(c(2, 0, -1, 1, 0), -c(2, 0, -1, 1, 0)),
            lambda: s96(c(2, 2, 1, 1, 2), -c(2, 2, 1, 1, 2)),
        ]
        for i in slots:
            a_ref[i, G * j:G * (j + 1), :] = fns[i]().astype(BF16)


class _Operands:
    def __init__(self, ref=None):
        self.ref = ref
        self.rows = {}

    def put(self, r0, v):
        if self.ref is None:
            self.rows[r0] = v
        else:
            self.ref[r0:r0 + G, :] = v.astype(BF16)

    def get(self, parts):
        if self.ref is None:
            vs = [self.rows[r] for r0, n in parts for r in range(r0, r0 + n, G)]
            return jnp.concatenate(vs, axis=0).astype(BF16)
        return jnp.concatenate([self.ref[r0:r0 + n, :] for r0, n in parts], axis=0)


class _Stats:
    def __init__(self, x_view):
        self.x = x_view
        self.p0 = jnp.broadcast_to(x_view[0:G, :].astype(F32)[0:1], (8, W2))
        self.p = self.p0
        self.s = None
        self.q = None
        self.k = 0

    def step(self, n):
        for _ in range(n):
            x = self.x[self.k * G:(self.k + 1) * G, :].astype(F32)
            for h in range(2):
                d = x[8 * h:8 * h + 8] - self.p
                self.s = d if self.s is None else self.s + d
                self.q = d * d if self.q is None else self.q + d * d
            self.k += 1

    def finish(self):
        s = jnp.sum(self.s, axis=0, keepdims=True) * (1.0 / D)
        q = jnp.sum(self.q, axis=0, keepdims=True) * (1.0 / D)
        var = jnp.maximum(q - s * s, 0.0)
        return self.p0[0:1] + s, jax.lax.rsqrt(var + EPS)


def _prep_tile(x_view, ops, cur, nxt_view, tick, t0, t1):
    def zz_at(t):
        z = tick(t)
        return jnp.concatenate([z, z], axis=1)

    if cur is None:
        st = _Stats(x_view)
        tm = t0 + (t1 - t0) * (0.33 if nxt_view is not None else 0.5)
        for k in range(12):
            if tick is not None:
                st.p = _link(st.p0, zz_at(t0 + (tm - t0) * k / 12))
            st.step(3)
        cur = st.finish()
        t0 = tm
    m = jnp.broadcast_to(cur[0], (8, W2))
    r = jnp.broadcast_to(cur[1], (G, W2))
    st = None if nxt_view is None else _Stats(nxt_view)

    for k in range(NPIECE):
        mm = m
        if tick is not None:
            zz = zz_at(t0 + (t1 - t0) * k / NPIECE)
            mm = _link(m, zz)
            if st is not None:
                st.p = _link(st.p0, zz)

        def nrm(r0, mm=jnp.concatenate([mm, mm], axis=0)):
            y = (x_view[r0:r0 + G, :].astype(F32) - mm) * r
            return y[:, :T], y[:, T:]

        if st is not None:
            st.step(STAT_STEPS[k])
        if k < 16:
            r0 = (k // 8) * 256 + (k % 8) * G
            b11, b12 = nrm(r0)
            b21, b22 = nrm(r0 + 128)
            pm = jnp.add if k % 8 < 6 else jnp.subtract
            vals = [pm(b11, b22), b11, b12 - b22, b21 - b11, b22, pm(b11, b12), pm(b21, b22)]
            for i, v in enumerate(vals):
                ops.put(i * 256 + k * G, v)
        else:
            r0 = (k - 16) * G
            b1, b2 = nrm(512 + r0)
            ops.put(SP + r0, b1 + b2)
            ops.put(SM + r0, b1 - b2)
    return None if st is None else st.finish()


def _mm_tile(ops, lhs_of, bias_ref, obuf, s, cols, plan, stored, bias_last=False):
    m = {}
    acc = [None] * 4
    for rnd in plan:
        for nm in rnd:
            rhs = ops.get(PASSES[nm])
            sl = ASLOT[nm]
            lhs = [lhs_of(sl + i) for i in range(rhs.shape[0] // 128)]
            m[nm] = _dot(jnp.concatenate(lhs, axis=1), rhs)
        for q in range(4):
            terms = [(nm, SIGMA[nm][q]) for nm in rnd if SIGMA[nm][q]]
            if not terms:
                continue
            s0 = terms[0][1]
            val = m[terms[0][0]]
            for nm, sg in terms[1:]:
                val = val + m[nm] if sg * s0 > 0 else val - m[nm]
            if acc[q] is None and bias_last:
                acc[q] = val if s0 > 0 else -val
                continue
            prev = acc[q] if acc[q] is not None else (bias_ref[:NH, :] if q < 2 else bias_ref[NH:, :])
            acc[q] = prev + val if s0 > 0 else prev - val
    if bias_last:
        acc = [acc[q] + (bias_ref[:NH, :] if q < 2 else bias_ref[NH:, :]) for q in range(4)]
    for h in range(2):
        obuf[2 * s + h, :, cols] = jnp.concatenate(acc[2 * h:2 * h + 2], axis=1).astype(BF16)
        if stored is not None:
            stored(h)
    return m


def _write_runs(groups, nhead, tpi, tau_w, lead):
    runs = {}
    h0 = 0
    for n in groups:
        tau = max(tau_w + max(h0 - lead, 0), 2 * (h0 + n))
        i, u = divmod(tau - nhead, tpi)
        lst = runs.setdefault(u, [])
        prev = lst[-1] if lst else None
        if prev and prev[1] == i - 1 and prev[4] == n and prev[3] in (None, (h0 - prev[2]) / (i - prev[0])):
            lst[-1] = (prev[0], i, prev[2], (h0 - prev[2]) // (i - prev[0]), n)
        else:
            lst.append((i, i, h0, None, n))
        h0 += n
    return runs


def _body(x_hbm, g_hbm, b_hbm, w_hbm, o_hbm, xbuf, obuf, wbuf, gbuf, bbuf, wt_ref, tmp_ref, a_ref,
          bias_ref, pa, pb, z_ref, isem, osem, *, U, head, groups, tau_w, lead, spans, strips):
    S, _, B = x_hbm.shape
    NT = B // W2
    nhead = sum(head)
    hs = nhead // NT
    NIT = (S - hs) // U
    TPI = U * NT
    pbuf = (pa, pb)

    def rd_cols(s, t0, n, k):
        return pltpu.make_async_copy(
            x_hbm.at[s, :, pl.ds(t0 * W2, n * W2)], xbuf.at[s, :, pl.ds(t0 * W2, n * W2)], isem.at[k])

    def rd(s0, n, k):
        return pltpu.make_async_copy(x_hbm.at[pl.ds(s0, n)], xbuf.at[pl.ds(s0, n)], isem.at[k])

    def wr(h0, n, segs):
        for j in segs:
            idx = (pl.ds(h0, n), pl.ds(j * SEG, SEG))
            pltpu.make_async_copy(obuf.at[idx], o_hbm.at[idx], osem.at[0]).start()

    def wr_cols(h0, n, cols):
        idx = (pl.ds(h0, n), slice(None), cols)
        pltpu.make_async_copy(obuf.at[idx], o_hbm.at[idx], osem.at[0]).start()

    def tile(s, t):
        return xbuf.at[s, :, pl.ds(t * W2, W2)]

    def rd_w(bi, k):
        rows = pl.ds(128 * bi, min(128, D - 128 * bi))
        return pltpu.make_async_copy(w_hbm.at[rows], wbuf.at[rows], isem.at[k])

    first = [pltpu.make_async_copy(g_hbm, gbuf, isem.at[0]), pltpu.make_async_copy(b_hbm, bbuf, isem.at[0])]
    w_rd = [[rd_w(bi, k) for bi in bis] for k, (bis, _) in enumerate(W_STEPS)]
    kx = len(W_STEPS)
    x0 = rd_cols(0, 0, 1, kx)

    def rd_tiles(lo, hi, k):
        cps = []
        while lo < hi:
            s, t = divmod(lo, NT)
            n = (hi - lo) // NT * NT if t == 0 and hi - lo >= NT else min(NT - t, hi - lo)
            cps.append(rd(s, n // NT, k) if t == 0 and n >= NT else rd_cols(s, t, n, k))
            lo += n
        return cps

    ends = [2] + [sum(head[:bi + 1]) + 2 for bi in range(1, len(head))]
    ends += [min(nhead + TPI * (i + 1) + 2, S * NT) for i in range(NIT)]
    chunks = [rd_tiles(lo, hi, kx + 1 + k) for k, (lo, hi) in enumerate(zip([1] + ends, ends))]
    head_waits = chunks[:len(head)]
    k0 = kx + 1 + len(head)
    for cp in first + sum(w_rd, []) + [x0] + sum(chunks, []):
        cp.start()

    for cp in first:
        cp.wait()
    gt = None
    for cps, (bis, slots) in zip(w_rd, W_STEPS):
        for cp in cps:
            cp.wait()
        _transpose_w(wbuf, wt_ref, bis)
        if gt is None:
            g = jnp.broadcast_to(gbuf[...].astype(F32).reshape(1, D), (G, D))
            gt = [g[:, 128 * i:128 * (i + 1)] for i in range(4)]
            gt.append(0.5 * jnp.concatenate([g[:, st:st + ln] for st, ln in BLOCKS[4]], axis=1))
        _prep_a(gt, wt_ref, tmp_ref, slots)
    brow = _dot(jnp.broadcast_to(bbuf[...].reshape(1, D), (16, D)), wbuf[...])[0:1]
    x0.wait()
    z_ref[...] = jnp.zeros(z_ref.shape, U32)
    _prep_tile(tile(0, 0), _Operands(pbuf[0]), None, None, None, 0, 0)
    _prep_a(gt, wt_ref, tmp_ref, [i for i in range(16) if not any(i in sl for _, sl in W_STEPS)])

    def block(st, s0, t0, n, pin, pout, stored=None, first=False):
        def lhs_of(i):
            if not first:
                return _upk(a_ref[i])
            v = tmp_ref[i]
            a_ref[i] = _bits(v)
            return v

        z = z_ref[...]
        ops = _Operands(pin)
        for u in range(n):
            tt = t0 + u
            ds, t = divmod(tt, NT)

            def view(q):
                d2, t2 = divmod(q, NT)
                s2 = s0 + d2
                if not isinstance(s2, int) and d2 == U:
                    s2 = jnp.minimum(s2, S - 1)
                return tile(s2, t2)

            m = _mm_tile(ops, lhs_of, bias_ref, obuf, s0 + ds, pl.ds(t * W2, W2), PLAN,
                         stored and functools.partial(stored, tt), first)

            def tick(tm, m=m):
                return _bits(m[PLAN[int(tm // NH)][0]][int(tm % NH) // 8 * 8:][:8]) & z

            ops = _Operands(pout if u == n - 1 else None)
            st = _prep_tile(view(tt + 1), ops, st, None if first else view(tt + 2), tick,
                            0, spans[0] if u < n - 1 else spans[1])
        return st

    pos = 0
    cur = 0
    st = None
    for bi, (n, cps) in enumerate(zip(head, head_waits)):
        for cp in cps:
            cp.wait()
        if bi == 0:
            bias_ref[...] = jnp.broadcast_to(brow, (T, D)).T
        nxt = cur if n > 1 else 1 - cur
        st = block(st, 0, pos, n, pbuf[cur], pbuf[nxt], first=bi == 0)
        cur = nxt
        pos += n

    runs = _write_runs(groups, nhead, TPI, tau_w, lead)

    def it(i, st):
        last = i == NIT - 1

        @pl.when(jnp.logical_not(last))
        def _():
            s1 = hs + i * U
            rd_cols(s1, 2, NT - 2, k0 + i).wait()
            rd(s1 + 1, U - 1, k0 + i).wait()
            rd_cols(s1 + U, 0, 2, k0 + i).wait()

        @pl.when(last)
        def _():
            for cp in chunks[-1]:
                cp.wait()

        def issue(u, part):
            half = NH // SEG // 2
            for i0, i1, hh, dh, n in runs.get(u, []):
                @pl.when(jnp.logical_and(i >= i0, i <= i1))
                def _():
                    wr(hh if dh is None else hh + dh * (i - i0), n, range(part * half, (part + 1) * half))

        def stored(tt, h):
            if h == 0:
                issue(tt, 1)
            elif tt + 1 < TPI:
                issue(tt + 1, 0)
            back = TPI - 1 - tt
            strip = strips[back] if back < len(strips) else 0
            if strip and (h == 1 or back == 0):
                @pl.when(last)
                def _():
                    h0 = 2 * (S - 1 - back // NT)
                    cols = pl.ds((tt % NT + 1 - strip) * W2, strip * W2)
                    if back == 0:
                        wr_cols(h0 + h, 1, cols)
                    else:
                        wr_cols(h0, 2, cols)

        issue(0, 0)
        return block(st, hs + i * U, 0, TPI, pbuf[cur], pbuf[cur], stored)

    jax.lax.fori_loop(0, NIT, it, st)
    pltpu.make_async_copy(obuf, o_hbm, osem.at[0]).wait()


def _run(x, g, b, w, U=4, head=(1, 1, 2, 4, 8), groups=(8,) * 6 + (4, 4, 2, 2), tau_w=62, lead=4,
         spans=(930, 1050), strips=(1, 1, 1, 1, 2, 0, 2)):
    B, S, _ = x.shape
    xt = jnp.transpose(x, (1, 2, 0))
    oshape = (2 * S, NH, B)
    nsem = len(W_STEPS) + 1 + len(head) + (S - sum(head) * W2 // B) // U
    out = pl.pallas_call(
        functools.partial(_body, U=U, head=head, groups=groups, tau_w=tau_w, lead=lead, spans=spans,
                          strips=strips),
        in_specs=[pl.BlockSpec(memory_space=pl.ANY)] * 4,
        out_specs=pl.BlockSpec(memory_space=pl.ANY),
        out_shape=jax.ShapeDtypeStruct(oshape, x.dtype),
        scratch_shapes=[
            pltpu.VMEM((S, D, B), BF16),
            pltpu.VMEM(oshape, BF16),
            pltpu.VMEM((D, D), BF16),
            pltpu.VMEM((D,), BF16),
            pltpu.VMEM((D,), BF16),
            pltpu.VMEM((5, D // 2, 128), U32),
            pltpu.VMEM((16, NH, 128), BF16),
            pltpu.VMEM((16, NH // 2, 128), U32),
            pltpu.VMEM((D, T), F32),
            pltpu.VMEM((PROWS, T), BF16),
            pltpu.VMEM((PROWS, T), BF16),
            pltpu.VMEM((8, T), U32),
            pltpu.SemaphoreType.DMA((nsem,)),
            pltpu.SemaphoreType.DMA((1,)),
        ],
        compiler_params=pltpu.CompilerParams(
            vmem_limit_bytes=110 * 1024 * 1024,
            disable_bounds_checks=True,
            disable_semaphore_checks=True,
        ),
    )(xt, g, b, w)
    return jnp.transpose(out.reshape(S, D, B), (2, 0, 1))


@jax.jit
def pallas_standalone__layernorm_linear__sampling_kernel(x, g, b, w):
    return _run(x, g, b, w)
```

```python
import functools

import jax
import jax.numpy as jnp
import jax.experimental.pallas as pl
import jax.experimental.pallas.tpu as pltpu

EPS = 1e-5
F32 = jnp.float32
BF16 = jnp.bfloat16
U32 = jnp.uint32

D = 576
G = 16
T = 128
W2 = 2 * T
NH = D // 2
SEG = 16
PROWS = 7 * 256 + 128
SP, SM = 7 * 256, 7 * 256 + 64


def _rows(i, lo, hi):
    return (i - 1) * 256 + lo, hi - lo


PASSES = {
    'I': [_rows(1, 0, 96), _rows(1, 224, 256)],
    'Z': [_rows(1, 128, 224), _rows(1, 96, 128)],
    'se1': [_rows(4, 0, 128)], 'de1': [_rows(4, 128, 256)],
    'se2': [_rows(3, 0, 128)], 'de2': [_rows(3, 128, 256)],
    'e1s': [(SP, 64), _rows(5, 96, 128), _rows(5, 224, 256)],
    'e2s': [(SP, 64), _rows(2, 96, 128), _rows(2, 224, 256)],
    'e1d': [_rows(5, 0, 96), (SM, 32), _rows(5, 128, 224), (SM + 32, 32)],
    'e2d': [_rows(2, 0, 96), (SM, 32), _rows(2, 128, 224), (SM + 32, 32)],
    'e11': [_rows(7, 0, 256)], 'e22': [_rows(6, 0, 256)],
}
SIGMA = {'I': (1, 0, 0, 1), 'Z': (1, 0, 0, -1), 'se1': (1, 0, 1, 0), 'de1': (1, 0, -1, 0),
         'se2': (0, 1, 0, 1), 'de2': (0, 1, 0, -1), 'e1s': (1, 1, 0, 0), 'e1d': (1, -1, 0, 0),
         'e2s': (0, 0, 1, 1), 'e2d': (0, 0, 1, -1), 'e11': (1, 0, 0, 0), 'e22': (0, 0, 0, 1)}
ASLOT = {'I': 0, 'Z': 1, 'se1': 2, 'de1': 3, 'se2': 4, 'de2': 5, 'e1s': 6, 'e2s': 7,
         'e1d': 8, 'e2d': 10, 'e11': 12, 'e22': 14}
PLAN = [['I', 'se1', 'de1', 'e2s'], ['e1d', 'e11'], ['Z', 'se2', 'de2', 'e1s'], ['e2d', 'e22']]
NPIECE = 20
OFFS = (0, 0.5, 0.25, 0.75)
STAT_STEPS = [2] * 16 + [1] * 4
BLOCKS = [[(0, 128)], [(128, 128)], [(256, 128)], [(384, 128)], [(512, 64), (544, 32), (512, 32)]]
W_STEPS = [([4, 1, 3], []), ([0, 2], [2, 3, 12, 13, 4, 5, 14, 15])]


def _dot(a, b):
    return jnp.dot(a, b, preferred_element_type=F32)


def _upk(v):
    return pltpu.bitcast(v, BF16)


def _bits(v):
    return pltpu.bitcast(v, U32)


def _link(v, zero):
    return pltpu.bitcast(_bits(v) | zero, F32)


def _transpose_w(w_ref, wt_ref, blocks):
    for bi in blocks:
        for c in range(5):
            wd = min(128, D - 128 * c)
            rows = [w_ref[st:st + ln, 128 * c:128 * c + wd] for st, ln in BLOCKS[bi]]
            wp = jnp.concatenate(rows, axis=0) if len(rows) > 1 else rows[0]
            wt_ref[bi, 64 * c:64 * c + wd // 2, :] = _bits(wp.T)


def _prep_a(gt, wt_ref, a_ref, slots):
    lane = jax.lax.broadcasted_iota(jnp.int32, (G, 128), 1)

    def s96(a, b):
        return jnp.where(lane < 96, a, b)

    def es(sv, sx, sy):
        return jnp.where(lane < 64, sv, s96(pltpu.roll(sx, 96, 1), sy))

    for j in range(NH // G):
        memo = {}

        def n(h, bi):
            if (h, bi) not in memo:
                r0 = 8 * (j + (h - 1) * (NH // G))
                memo[(h, bi)] = gt[bi] * _upk(wt_ref[bi, r0:r0 + 8, :]).astype(F32)
            return memo[(h, bi)]

        def c(h1, b1, sg, h2, b2):
            key = (h1, b1, sg, h2, b2)
            if key not in memo:
                memo[key] = n(h1, b1) + n(h2, b2) if sg > 0 else n(h1, b1) - n(h2, b2)
            return memo[key]

        fns = [
            lambda: s96(c(1, 0, 1, 2, 1), c(1, 2, -1, 2, 3)),
            lambda: s96(c(1, 2, -1, 2, 3), c(1, 0, 1, 2, 1)),
            lambda: n(2, 1), lambda: -n(2, 3), lambda: n(1, 0), lambda: n(1, 2),
            lambda: es(n(1, 4), c(1, 0, 1, 1, 1), c(1, 2, 1, 1, 3)),
            lambda: es(n(2, 4), c(2, 0, 1, 2, 1), c(2, 2, 1, 2, 3)),
            lambda: s96(-c(1, 0, 1, 1, 1), n(1, 4)),
            lambda: s96(-c(1, 2, 1, 1, 3), pltpu.roll(n(1, 4), 32, 1)),
            lambda: s96(c(2, 0, 1, 2, 1), n(2, 4)),
            lambda: s96(c(2, 2, 1, 2, 3), pltpu.roll(n(2, 4), 32, 1)),
            lambda: c(1, 1, -1, 2, 1), lambda: c(1, 3, 1, 2, 3),
            lambda: s96(c(2, 0, -1, 1, 0), -c(2, 0, -1, 1, 0)),
            lambda: s96(c(2, 2, 1, 1, 2), -c(2, 2, 1, 1, 2)),
        ]
        for i in slots:
            a_ref[i, G * j:G * (j + 1), :] = fns[i]().astype(BF16)


class _Operands:
    def __init__(self, ref=None):
        self.ref = ref
        self.rows = {}

    def put(self, r0, v):
        if self.ref is None:
            self.rows[r0] = v
        else:
            self.ref[r0:r0 + G, :] = v.astype(BF16)

    def get(self, parts):
        if self.ref is None:
            vs = [self.rows[r] for r0, n in parts for r in range(r0, r0 + n, G)]
            return jnp.concatenate(vs, axis=0).astype(BF16)
        return jnp.concatenate([self.ref[r0:r0 + n, :] for r0, n in parts], axis=0)


class _Stats:
    def __init__(self, x_view):
        self.x = x_view
        self.p0 = jnp.broadcast_to(x_view[0:G, :].astype(F32)[0:1], (8, W2))
        self.p = self.p0
        self.s = None
        self.q = None
        self.k = 0

    def step(self, n):
        for _ in range(n):
            x = self.x[self.k * G:(self.k + 1) * G, :].astype(F32)
            for h in range(2):
                d = x[8 * h:8 * h + 8] - self.p
                self.s = d if self.s is None else self.s + d
                self.q = d * d if self.q is None else self.q + d * d
            self.k += 1

    def finish(self):
        s = jnp.sum(self.s, axis=0, keepdims=True) * (1.0 / D)
        q = jnp.sum(self.q, axis=0, keepdims=True) * (1.0 / D)
        var = jnp.maximum(q - s * s, 0.0)
        return self.p0[0:1] + s, jax.lax.rsqrt(var + EPS)


def _prep_tile(x_view, ops, cur, nxt_view, tick, t0, t1):
    def zz_at(t):
        z = tick(t)
        return jnp.concatenate([z, z], axis=1)

    if cur is None:
        st = _Stats(x_view)
        tm = t0 + (t1 - t0) * (0.33 if nxt_view is not None else 0.5)
        for k in range(12):
            if tick is not None:
                st.p = _link(st.p0, zz_at(t0 + (tm - t0) * k / 12))
            st.step(3)
        cur = st.finish()
        t0 = tm
    m = jnp.broadcast_to(cur[0], (8, W2))
    r = jnp.broadcast_to(cur[1], (G, W2))
    st = None if nxt_view is None else _Stats(nxt_view)

    for k in range(NPIECE):
        def lk(v, off):
            return v if tick is None else _link(v, zz_at(t0 + (t1 - t0) * (k + off) / NPIECE))

        memo = {}

        def nrm(r0, off=OFFS[0]):
            if off not in memo:
                mm = lk(m, off)
                memo[off] = jnp.concatenate([mm, mm], axis=0)
            y = (x_view[r0:r0 + G, :].astype(F32) - memo[off]) * r
            return y[:, :T], y[:, T:]

        if st is not None:
            for ss in range(STAT_STEPS[k]):
                st.p = lk(st.p0, OFFS[2 + ss])
                st.step(1)
        if k < 16:
            r0 = (k // 8) * 256 + (k % 8) * G
            b11, b12 = nrm(r0)
            b21, b22 = nrm(r0 + 128, OFFS[1])
            pm = jnp.add if k % 8 < 6 else jnp.subtract
            vals = [pm(b11, b22), b11, b12 - b22, b21 - b11, b22, pm(b11, b12), pm(b21, b22)]
            for i, v in enumerate(vals):
                ops.put(i * 256 + k * G, v)
        else:
            r0 = (k - 16) * G
            b1, b2 = nrm(512 + r0)
            ops.put(SP + r0, b1 + b2)
            ops.put(SM + r0, b1 - b2)
    return None if st is None else st.finish()


def _mm_tile(ops, lhs_of, bias_ref, obuf, s, cols, plan, stored, bias_last):
    m = {}
    acc = [None] * 4
    for rnd in plan:
        for nm in rnd:
            rhs = ops.get(PASSES[nm])
            sl = ASLOT[nm]
            lhs = [lhs_of(sl + i) for i in range(rhs.shape[0] // 128)]
            m[nm] = _dot(jnp.concatenate(lhs, axis=1), rhs)
        for q in range(4):
            terms = [(nm, SIGMA[nm][q]) for nm in rnd if SIGMA[nm][q]]
            if not terms:
                continue
            s0 = terms[0][1]
            val = m[terms[0][0]]
            for nm, sg in terms[1:]:
                val = val + m[nm] if sg * s0 > 0 else val - m[nm]
            if acc[q] is None and bias_last:
                acc[q] = val if s0 > 0 else -val
                continue
            prev = acc[q] if acc[q] is not None else (bias_ref[:NH, :] if q < 2 else bias_ref[NH:, :])
            acc[q] = prev + val if s0 > 0 else prev - val
    if bias_last:
        acc = [acc[q] + (bias_ref[:NH, :] if q < 2 else bias_ref[NH:, :]) for q in range(4)]
    for h in range(2):
        obuf[2 * s + h, :, cols] = jnp.concatenate(acc[2 * h:2 * h + 2], axis=1).astype(BF16)
        if stored is not None:
            stored(h)
    return m


def _write_runs(groups, nhead, tpi, tau_w, lead):
    runs = {}
    h0 = 0
    for n in groups:
        tau = max(tau_w + max(h0 - lead, 0), 2 * (h0 + n))
        i, u = divmod(tau - nhead, tpi)
        lst = runs.setdefault(u, [])
        prev = lst[-1] if lst else None
        if prev and prev[1] == i - 1 and prev[4] == n and prev[3] in (None, (h0 - prev[2]) / (i - prev[0])):
            lst[-1] = (prev[0], i, prev[2], (h0 - prev[2]) // (i - prev[0]), n)
        else:
            lst.append((i, i, h0, None, n))
        h0 += n
    return runs


def _body(x_hbm, g_hbm, b_hbm, w_hbm, o_hbm, xbuf, obuf, wbuf, gbuf, bbuf, wt_ref, tmp_ref, a_ref,
          bias_ref, pa, pb, z_ref, isem, osem, *, U, head, groups, tau_w, lead, spans, strips):
    S, _, B = x_hbm.shape
    NT = B // W2
    nhead = sum(head)
    hs = nhead // NT
    NIT = (S - hs) // U
    TPI = U * NT
    pbuf = (pa, pb)

    def rd_cols(s, t0, n, k):
        return pltpu.make_async_copy(
            x_hbm.at[s, :, pl.ds(t0 * W2, n * W2)], xbuf.at[s, :, pl.ds(t0 * W2, n * W2)], isem.at[k])

    def rd(s0, n, k):
        return pltpu.make_async_copy(x_hbm.at[pl.ds(s0, n)], xbuf.at[pl.ds(s0, n)], isem.at[k])

    def wr(h0, n, segs):
        for j in segs:
            idx = (pl.ds(h0, n), pl.ds(j * SEG, SEG))
            pltpu.make_async_copy(obuf.at[idx], o_hbm.at[idx], osem.at[0]).start()

    def wr_cols(h0, n, cols):
        idx = (pl.ds(h0, n), slice(None), cols)
        pltpu.make_async_copy(obuf.at[idx], o_hbm.at[idx], osem.at[0]).start()

    def tile(s, t):
        return xbuf.at[s, :, pl.ds(t * W2, W2)]

    def rd_w(bi, k):
        rows = pl.ds(128 * bi, min(128, D - 128 * bi))
        return pltpu.make_async_copy(w_hbm.at[rows], wbuf.at[rows], isem.at[k])

    first = [pltpu.make_async_copy(g_hbm, gbuf, isem.at[0]), pltpu.make_async_copy(b_hbm, bbuf, isem.at[0])]
    w_rd = [[rd_w(bi, k) for bi in bis] for k, (bis, _) in enumerate(W_STEPS)]
    kx = len(W_STEPS)
    x0 = rd_cols(0, 0, 1, kx)

    def rd_tiles(lo, hi, k):
        cps = []
        while lo < hi:
            s, t = divmod(lo, NT)
            n = (hi - lo) // NT * NT if t == 0 and hi - lo >= NT else min(NT - t, hi - lo)
            cps.append(rd(s, n // NT, k) if t == 0 and n >= NT else rd_cols(s, t, n, k))
            lo += n
        return cps

    ends = [sum(head[:bi + 1]) + (1 if bi == 0 else 2) for bi in range(len(head))]
    ends += [min(nhead + TPI * (i + 1) + 2, S * NT) for i in range(NIT)]
    chunks = [rd_tiles(lo, hi, kx + 1 + k) for k, (lo, hi) in enumerate(zip([1] + ends, ends))]
    head_waits = chunks[:len(head)]
    k0 = kx + 1 + len(head)
    for cp in first + sum(w_rd, []) + [x0] + sum(chunks, []):
        cp.start()

    for cp in first:
        cp.wait()
    gt = None
    for cps, (bis, slots) in zip(w_rd, W_STEPS):
        for cp in cps:
            cp.wait()
        _transpose_w(wbuf, wt_ref, bis)
        if gt is None:
            g = jnp.broadcast_to(gbuf[...].astype(F32).reshape(1, D), (G, D))
            gt = [g[:, 128 * i:128 * (i + 1)] for i in range(4)]
            gt.append(0.5 * jnp.concatenate([g[:, st:st + ln] for st, ln in BLOCKS[4]], axis=1))
        _prep_a(gt, wt_ref, tmp_ref, slots)
    brow = _dot(jnp.broadcast_to(bbuf[...].reshape(1, D), (16, D)), wbuf[...])[0:1]
    x0.wait()
    z_ref[...] = jnp.zeros(z_ref.shape, U32)
    _prep_tile(tile(0, 0), _Operands(pbuf[0]), None, None, None, 0, 0)
    _prep_a(gt, wt_ref, tmp_ref, [i for i in range(16) if not any(i in sl for _, sl in W_STEPS)])

    def block(st, s0, t0, n, pin, pout, stored=None, first=False):
        def lhs_of(i):
            if not first:
                return _upk(a_ref[i])
            v = tmp_ref[i]
            a_ref[i] = _bits(v)
            return v

        z = z_ref[...]
        ops = _Operands(pin)
        for u in range(n):
            tt = t0 + u
            ds, t = divmod(tt, NT)

            def view(q):
                d2, t2 = divmod(q, NT)
                s2 = s0 + d2
                if not isinstance(s2, int) and d2 == U:
                    s2 = jnp.minimum(s2, S - 1)
                return tile(s2, t2)

            m = _mm_tile(ops, lhs_of, bias_ref, obuf, s0 + ds, pl.ds(t * W2, W2), PLAN,
                         stored and functools.partial(stored, tt), first)

            def tick(tm, m=m):
                return _bits(m[PLAN[int(tm // NH)][0]][int(tm % NH) // 8 * 8:][:8]) & z

            ops = _Operands(pout if u == n - 1 else None)
            st = _prep_tile(view(tt + 1), ops, st, None if first else view(tt + 2), tick,
                            0, spans[0] if u < n - 1 else spans[1])
        return st

    pos = 0
    cur = 0
    st = None
    for bi, (n, cps) in enumerate(zip(head, head_waits)):
        for cp in cps:
            cp.wait()
        if bi == 0:
            bias_ref[...] = jnp.broadcast_to(brow, (T, D)).T
        nxt = cur if n > 1 else 1 - cur
        st = block(st, 0, pos, n, pbuf[cur], pbuf[nxt], first=bi == 0)
        cur = nxt
        pos += n

    runs = _write_runs(groups, nhead, TPI, tau_w, lead)

    def it(i, st):
        last = i == NIT - 1

        @pl.when(jnp.logical_not(last))
        def _():
            s1 = hs + i * U
            rd_cols(s1, 2, NT - 2, k0 + i).wait()
            rd(s1 + 1, U - 1, k0 + i).wait()
            rd_cols(s1 + U, 0, 2, k0 + i).wait()

        @pl.when(last)
        def _():
            for cp in chunks[-1]:
                cp.wait()

        def issue(u, part):
            half = NH // SEG // 2
            for i0, i1, hh, dh, n in runs.get(u, []):
                @pl.when(jnp.logical_and(i >= i0, i <= i1))
                def _():
                    wr(hh if dh is None else hh + dh * (i - i0), n, range(part * half, (part + 1) * half))

        def stored(tt, h):
            if h == 0:
                issue(tt, 1)
            elif tt + 1 < TPI:
                issue(tt + 1, 0)
            back = TPI - 1 - tt
            strip = strips[back] if back < len(strips) else 0
            if strip and (h == 1 or back == 0):
                @pl.when(last)
                def _():
                    h0 = 2 * (S - 1 - back // NT)
                    cols = pl.ds((tt % NT + 1 - strip) * W2, strip * W2)
                    if back == 0:
                        wr_cols(h0 + h, 1, cols)
                    else:
                        wr_cols(h0, 2, cols)

        issue(0, 0)
        return block(st, hs + i * U, 0, TPI, pbuf[cur], pbuf[cur], stored)

    jax.lax.fori_loop(0, NIT, it, st)
    pltpu.make_async_copy(obuf, o_hbm, osem.at[0]).wait()


def _run(x, g, b, w, U=4, head=(1, 1, 2, 4, 8), groups=(8,) * 6 + (4, 4, 2, 2), tau_w=61, lead=4,
         spans=(990, 1050), strips=(1, 1, 1, 1, 2, 0, 2)):
    B, S, _ = x.shape
    xt = jnp.transpose(x, (1, 2, 0))
    oshape = (2 * S, NH, B)
    nsem = len(W_STEPS) + 1 + len(head) + (S - sum(head) * W2 // B) // U
    out = pl.pallas_call(
        functools.partial(_body, U=U, head=head, groups=groups, tau_w=tau_w, lead=lead, spans=spans,
                          strips=strips),
        in_specs=[pl.BlockSpec(memory_space=pl.ANY)] * 4,
        out_specs=pl.BlockSpec(memory_space=pl.ANY),
        out_shape=jax.ShapeDtypeStruct(oshape, x.dtype),
        scratch_shapes=[
            pltpu.VMEM((S, D, B), BF16),
            pltpu.VMEM(oshape, BF16),
            pltpu.VMEM((D, D), BF16),
            pltpu.VMEM((D,), BF16),
            pltpu.VMEM((D,), BF16),
            pltpu.VMEM((5, D // 2, 128), U32),
            pltpu.VMEM((16, NH, 128), BF16),
            pltpu.VMEM((16, NH // 2, 128), U32),
            pltpu.VMEM((D, T), F32),
            pltpu.VMEM((PROWS, T), BF16),
            pltpu.VMEM((PROWS, T), BF16),
            pltpu.VMEM((8, T), U32),
            pltpu.SemaphoreType.DMA((nsem,)),
            pltpu.SemaphoreType.DMA((1,)),
        ],
        compiler_params=pltpu.CompilerParams(
            vmem_limit_bytes=110 * 1024 * 1024,
            disable_bounds_checks=True,
            disable_semaphore_checks=True,
        ),
    )(xt, g, b, w)
    return jnp.transpose(out.reshape(S, D, B), (2, 0, 1))


@jax.jit
def pallas_standalone__layernorm_linear__sampling_kernel(x, g, b, w):
    return _run(x, g, b, w)
```

```python
import functools

import jax
import jax.numpy as jnp
import jax.experimental.pallas as pl
import jax.experimental.pallas.tpu as pltpu

EPS = 1e-5
F32 = jnp.float32
BF16 = jnp.bfloat16
U32 = jnp.uint32

D = 576
G = 16
T = 128
W2 = 2 * T
NH = D // 2
SEG = 16
PROWS = 7 * 256 + 128
SP, SM = 7 * 256, 7 * 256 + 64


def _rows(i, lo, hi):
    return (i - 1) * 256 + lo, hi - lo


PASSES = {
    'I': [_rows(1, 0, 96), _rows(1, 224, 256)],
    'Z': [_rows(1, 128, 224), _rows(1, 96, 128)],
    'se1': [_rows(4, 0, 128)], 'de1': [_rows(4, 128, 256)],
    'se2': [_rows(3, 0, 128)], 'de2': [_rows(3, 128, 256)],
    'e1s': [(SP, 64), _rows(5, 96, 128), _rows(5, 224, 256)],
    'e2s': [(SP, 64), _rows(2, 96, 128), _rows(2, 224, 256)],
    'e1d': [_rows(5, 0, 96), (SM, 32), _rows(5, 128, 224), (SM + 32, 32)],
    'e2d': [_rows(2, 0, 96), (SM, 32), _rows(2, 128, 224), (SM + 32, 32)],
    'e11': [_rows(7, 0, 256)], 'e22': [_rows(6, 0, 256)],
}
SIGMA = {'I': (1, 0, 0, 1), 'Z': (1, 0, 0, -1), 'se1': (1, 0, 1, 0), 'de1': (1, 0, -1, 0),
         'se2': (0, 1, 0, 1), 'de2': (0, 1, 0, -1), 'e1s': (1, 1, 0, 0), 'e1d': (1, -1, 0, 0),
         'e2s': (0, 0, 1, 1), 'e2d': (0, 0, 1, -1), 'e11': (1, 0, 0, 0), 'e22': (0, 0, 0, 1)}
ASLOT = {'I': 0, 'Z': 1, 'se1': 2, 'de1': 3, 'se2': 4, 'de2': 5, 'e1s': 6, 'e2s': 7,
         'e1d': 8, 'e2d': 10, 'e11': 12, 'e22': 14}
PLAN = [['I', 'se1', 'de1', 'e2s'], ['e1d', 'e11'], ['Z', 'se2', 'de2', 'e1s'], ['e2d', 'e22']]
NPIECE = 20
OFFS = (0, 0.5, 0.25, 0.75)
STAT_STEPS = [2] * 16 + [1] * 4
BLOCKS = [[(0, 128)], [(128, 128)], [(256, 128)], [(384, 128)], [(512, 64), (544, 32), (512, 32)]]
W_STEPS = [([4, 1, 3], []), ([0, 2], [2, 3, 12, 13, 4, 5, 14, 15])]


def _dot(a, b):
    return jnp.dot(a, b, preferred_element_type=F32)


def _upk(v):
    return pltpu.bitcast(v, BF16)


def _bits(v):
    return pltpu.bitcast(v, U32)


def _link(v, zero):
    return pltpu.bitcast(_bits(v) | zero, F32)


def _transpose_w(w_ref, wt_ref, blocks):
    for bi in blocks:
        for c in range(5):
            wd = min(128, D - 128 * c)
            rows = [w_ref[st:st + ln, 128 * c:128 * c + wd] for st, ln in BLOCKS[bi]]
            wp = jnp.concatenate(rows, axis=0) if len(rows) > 1 else rows[0]
            wt_ref[bi, 64 * c:64 * c + wd // 2, :] = _bits(wp.T)


def _prep_a(gt, wt_ref, a_ref, slots):
    lane = jax.lax.broadcasted_iota(jnp.int32, (G, 128), 1)

    def s96(a, b):
        return jnp.where(lane < 96, a, b)

    def es(sv, sx, sy):
        return jnp.where(lane < 64, sv, s96(pltpu.roll(sx, 96, 1), sy))

    for j in range(NH // G):
        memo = {}

        def n(h, bi):
            if (h, bi) not in memo:
                r0 = 8 * (j + (h - 1) * (NH // G))
                memo[(h, bi)] = gt[bi] * _upk(wt_ref[bi, r0:r0 + 8, :]).astype(F32)
            return memo[(h, bi)]

        def c(h1, b1, sg, h2, b2):
            key = (h1, b1, sg, h2, b2)
            if key not in memo:
                memo[key] = n(h1, b1) + n(h2, b2) if sg > 0 else n(h1, b1) - n(h2, b2)
            return memo[key]

        fns = [
            lambda: s96(c(1, 0, 1, 2, 1), c(1, 2, -1, 2, 3)),
            lambda: s96(c(1, 2, -1, 2, 3), c(1, 0, 1, 2, 1)),
            lambda: n(2, 1), lambda: -n(2, 3), lambda: n(1, 0), lambda: n(1, 2),
            lambda: es(n(1, 4), c(1, 0, 1, 1, 1), c(1, 2, 1, 1, 3)),
            lambda: es(n(2, 4), c(2, 0, 1, 2, 1), c(2, 2, 1, 2, 3)),
            lambda: s96(-c(1, 0, 1, 1, 1), n(1, 4)),
            lambda: s96(-c(1, 2, 1, 1, 3), pltpu.roll(n(1, 4), 32, 1)),
            lambda: s96(c(2, 0, 1, 2, 1), n(2, 4)),
            lambda: s96(c(2, 2, 1, 2, 3), pltpu.roll(n(2, 4), 32, 1)),
            lambda: c(1, 1, -1, 2, 1), lambda: c(1, 3, 1, 2, 3),
            lambda: s96(c(2, 0, -1, 1, 0), -c(2, 0, -1, 1, 0)),
            lambda: s96(c(2, 2, 1, 1, 2), -c(2, 2, 1, 1, 2)),
        ]
        for i in slots:
            a_ref[i, G * j:G * (j + 1), :] = fns[i]().astype(BF16)


class _Operands:
    def __init__(self, ref=None):
        self.ref = ref
        self.rows = {}

    def put(self, r0, v):
        if self.ref is None:
            self.rows[r0] = v
        else:
            self.ref[r0:r0 + G, :] = v.astype(BF16)

    def get(self, parts):
        if self.ref is None:
            vs = [self.rows[r] for r0, n in parts for r in range(r0, r0 + n, G)]
            return jnp.concatenate(vs, axis=0).astype(BF16)
        return jnp.concatenate([self.ref[r0:r0 + n, :] for r0, n in parts], axis=0)


class _Stats:
    def __init__(self, x_view):
        self.x = x_view
        self.p0 = jnp.broadcast_to(x_view[0:G, :].astype(F32)[0:1], (8, W2))
        self.p = self.p0
        self.s = None
        self.q = None
        self.k = 0

    def step(self, n):
        for _ in range(n):
            x = self.x[self.k * G:(self.k + 1) * G, :].astype(F32)
            for h in range(2):
                d = x[8 * h:8 * h + 8] - self.p
                self.s = d if self.s is None else self.s + d
                self.q = d * d if self.q is None else self.q + d * d
            self.k += 1

    def finish(self):
        s = jnp.sum(self.s, axis=0, keepdims=True) * (1.0 / D)
        q = jnp.sum(self.q, axis=0, keepdims=True) * (1.0 / D)
        var = jnp.maximum(q - s * s, 0.0)
        return self.p0[0:1] + s, jax.lax.rsqrt(var + EPS)


def _prep_tile(x_view, ops, cur, nxt_view, tick, t0, t1):
    def zz_at(t):
        z = tick(t)
        return jnp.concatenate([z, z], axis=1)

    if cur is None:
        st = _Stats(x_view)
        tm = t0 + (t1 - t0) * (0.33 if nxt_view is not None else 0.5)
        for k in range(12):
            if tick is not None:
                st.p = _link(st.p0, zz_at(t0 + (tm - t0) * k / 12))
            st.step(3)
        cur = st.finish()
        t0 = tm
    m = jnp.broadcast_to(cur[0], (8, W2))
    r = jnp.broadcast_to(cur[1], (G, W2))
    st = None if nxt_view is None else _Stats(nxt_view)

    for k in range(NPIECE):
        def lk(v, off):
            return v if tick is None else _link(v, zz_at(t0 + (t1 - t0) * (k + off) / NPIECE))

        memo = {}

        def nrm(r0, off=OFFS[0]):
            if off not in memo:
                mm = lk(m, off)
                memo[off] = jnp.concatenate([mm, mm], axis=0)
            y = (x_view[r0:r0 + G, :].astype(F32) - memo[off]) * r
            return y[:, :T], y[:, T:]

        if st is not None:
            for ss in range(STAT_STEPS[k]):
                st.p = lk(st.p0, OFFS[2 + ss])
                st.step(1)
        if k < 16:
            r0 = (k // 8) * 256 + (k % 8) * G
            b11, b12 = nrm(r0)
            b21, b22 = nrm(r0 + 128, OFFS[1])
            pm = jnp.add if k % 8 < 6 else jnp.subtract
            vals = [pm(b11, b22), b11, b12 - b22, b21 - b11, b22, pm(b11, b12), pm(b21, b22)]
            for i, v in enumerate(vals):
                ops.put(i * 256 + k * G, v)
        else:
            r0 = (k - 16) * G
            b1, b2 = nrm(512 + r0)
            ops.put(SP + r0, b1 + b2)
            ops.put(SM + r0, b1 - b2)
    return None if st is None else st.finish()


def _mm_tile(ops, lhs_of, bias_ref, obuf, s, cols, plan, stored, bias_last):
    m = {}
    acc = [None] * 4
    for rnd in plan:
        for nm in rnd:
            rhs = ops.get(PASSES[nm])
            sl = ASLOT[nm]
            lhs = [lhs_of(sl + i) for i in range(rhs.shape[0] // 128)]
            m[nm] = _dot(jnp.concatenate(lhs, axis=1), rhs)
        for q in range(4):
            terms = [(nm, SIGMA[nm][q]) for nm in rnd if SIGMA[nm][q]]
            if not terms:
                continue
            s0 = terms[0][1]
            val = m[terms[0][0]]
            for nm, sg in terms[1:]:
                val = val + m[nm] if sg * s0 > 0 else val - m[nm]
            if acc[q] is None and bias_last:
                acc[q] = val if s0 > 0 else -val
                continue
            prev = acc[q] if acc[q] is not None else (bias_ref[:NH, :] if q < 2 else bias_ref[NH:, :])
            acc[q] = prev + val if s0 > 0 else prev - val
    if bias_last:
        acc = [acc[q] + (bias_ref[:NH, :] if q < 2 else bias_ref[NH:, :]) for q in range(4)]
    for h in range(2):
        obuf[2 * s + h, :, cols] = jnp.concatenate(acc[2 * h:2 * h + 2], axis=1).astype(BF16)
        if stored is not None:
            stored(h)
    return m


def _write_runs(groups, nhead, tpi, tau_w, lead):
    runs = {}
    h0 = 0
    for n in groups:
        tau = max(tau_w + max(h0 - lead, 0), 2 * (h0 + n))
        i, u = divmod(tau - nhead, tpi)
        lst = runs.setdefault(u, [])
        prev = lst[-1] if lst else None
        if prev and prev[1] == i - 1 and prev[4] == n and prev[3] in (None, (h0 - prev[2]) / (i - prev[0])):
            lst[-1] = (prev[0], i, prev[2], (h0 - prev[2]) // (i - prev[0]), n)
        else:
            lst.append((i, i, h0, None, n))
        h0 += n
    return runs


def _body(x_hbm, g_hbm, b_hbm, w_hbm, o_hbm, xbuf, obuf, wbuf, gbuf, bbuf, wt_ref, tmp_ref, a_ref,
          bias_ref, pa, pb, z_ref, isem, osem, *, head, loops, groups, tau_w, lead, spans, strips):
    S, _, B = x_hbm.shape
    NT = B // W2
    pbuf = (pa, pb)

    def rd_cols(s, t0, n, k):
        return pltpu.make_async_copy(
            x_hbm.at[s, :, pl.ds(t0 * W2, n * W2)], xbuf.at[s, :, pl.ds(t0 * W2, n * W2)], isem.at[k])

    def rd(s0, n, k):
        return pltpu.make_async_copy(x_hbm.at[pl.ds(s0, n)], xbuf.at[pl.ds(s0, n)], isem.at[k])

    def wr(h0, n, segs):
        for j in segs:
            idx = (pl.ds(h0, n), pl.ds(j * SEG, SEG))
            pltpu.make_async_copy(obuf.at[idx], o_hbm.at[idx], osem.at[0]).start()

    def wr_cols(h0, n, cols):
        idx = (pl.ds(h0, n), slice(None), cols)
        pltpu.make_async_copy(obuf.at[idx], o_hbm.at[idx], osem.at[0]).start()

    def tile(s, t):
        return xbuf.at[s, :, pl.ds(t * W2, W2)]

    def rd_w(bi, k):
        rows = pl.ds(128 * bi, min(128, D - 128 * bi))
        return pltpu.make_async_copy(w_hbm.at[rows], wbuf.at[rows], isem.at[k])

    first = [pltpu.make_async_copy(g_hbm, gbuf, isem.at[0]), pltpu.make_async_copy(b_hbm, bbuf, isem.at[0])]
    w_rd = [[rd_w(bi, k) for bi in bis] for k, (bis, _) in enumerate(W_STEPS)]
    kx = len(W_STEPS)
    x0 = rd_cols(0, 0, 1, kx)

    def rd_tiles(lo, hi, k):
        cps = []
        while lo < hi:
            s, t = divmod(lo, NT)
            n = (hi - lo) // NT * NT if t == 0 and hi - lo >= NT else min(NT - t, hi - lo)
            cps.append(rd(s, n // NT, k) if t == 0 and n >= NT else rd_cols(s, t, n, k))
            lo += n
        return cps

    sizes = list(head) + [u * NT for u, reps in loops for _ in range(reps)]
    ends = [min(sum(sizes[:bi + 1]) + (1 if bi == 0 else 2), S * NT) for bi in range(len(sizes))]
    chunks = [rd_tiles(lo, hi, kx + 1 + k) for k, (lo, hi) in enumerate(zip([1] + ends, ends))]
    for cp in first + sum(w_rd, []) + [x0] + sum(chunks, []):
        cp.start()

    for cp in first:
        cp.wait()
    gt = None
    for cps, (bis, slots) in zip(w_rd, W_STEPS):
        for cp in cps:
            cp.wait()
        _transpose_w(wbuf, wt_ref, bis)
        if gt is None:
            g = jnp.broadcast_to(gbuf[...].astype(F32).reshape(1, D), (G, D))
            gt = [g[:, 128 * i:128 * (i + 1)] for i in range(4)]
            gt.append(0.5 * jnp.concatenate([g[:, st:st + ln] for st, ln in BLOCKS[4]], axis=1))
        _prep_a(gt, wt_ref, tmp_ref, slots)
    brow = _dot(jnp.broadcast_to(bbuf[...].reshape(1, D), (16, D)), wbuf[...])[0:1]
    x0.wait()
    z_ref[...] = jnp.zeros(z_ref.shape, U32)
    _prep_tile(tile(0, 0), _Operands(pbuf[0]), None, None, None, 0, 0)
    _prep_a(gt, wt_ref, tmp_ref, [i for i in range(16) if not any(i in sl for _, sl in W_STEPS)])

    def block(st, s0, t0, n, pin, pout, stored=None, first=False):
        def lhs_of(i):
            if not first:
                return _upk(a_ref[i])
            v = tmp_ref[i]
            a_ref[i] = _bits(v)
            return v

        z = z_ref[...]
        ops = _Operands(pin)
        for u in range(n):
            tt = t0 + u
            ds, t = divmod(tt, NT)

            def view(q):
                d2, t2 = divmod(q, NT)
                s2 = s0 + d2
                if not isinstance(s2, int) and q >= n:
                    s2 = jnp.minimum(s2, S - 1)
                return tile(s2, t2)

            m = _mm_tile(ops, lhs_of, bias_ref, obuf, s0 + ds, pl.ds(t * W2, W2), PLAN,
                         stored and functools.partial(stored, tt), first)

            def tick(tm, m=m):
                return _bits(m[PLAN[int(tm // NH)][0]][int(tm % NH) // 8 * 8:][:8]) & z

            ops = _Operands(pout if u == n - 1 else None)
            st = _prep_tile(view(tt + 1), ops, st, None if first else view(tt + 2), tick,
                            0, spans[0] if u < n - 1 else spans[1])
        return st

    pos = 0
    cur = 0
    st = None
    for bi, (n, cps) in enumerate(zip(head, chunks)):
        for cp in cps:
            cp.wait()
        if bi == 0:
            bias_ref[...] = jnp.broadcast_to(brow, (T, D)).T
        nxt = cur if n > 1 else 1 - cur
        st = block(st, 0, pos, n, pbuf[cur], pbuf[nxt], first=bi == 0)
        cur = nxt
        pos += n

    def loop(st, hs, U, NIT, k0, final):
        TPI = U * NT
        runs = _write_runs(groups, hs * NT, TPI, tau_w, lead) if final else {}

        def it(i, st):
            last = i == NIT - 1

            def wait_chunk():
                s1 = hs + i * U
                rd_cols(s1, 2, NT - 2, k0 + i).wait()
                rd(s1 + 1, U - 1, k0 + i).wait()
                rd_cols(s1 + U, 0, 2, k0 + i).wait()

            if final:
                pl.when(jnp.logical_not(last))(wait_chunk)

                @pl.when(last)
                def _():
                    for cp in chunks[-1]:
                        cp.wait()
            else:
                wait_chunk()

            def issue(u, part):
                half = NH // SEG // 2
                for i0, i1, hh, dh, n in runs.get(u, []):
                    @pl.when(jnp.logical_and(i >= i0, i <= i1))
                    def _():
                        wr(hh if dh is None else hh + dh * (i - i0), n, range(part * half, (part + 1) * half))

            def stored(tt, h):
                if h == 0:
                    issue(tt, 1)
                elif tt + 1 < TPI:
                    issue(tt + 1, 0)
                back = TPI - 1 - tt
                strip = strips[back] if back < len(strips) else 0
                if strip and (h == 1 or back == 0):
                    @pl.when(last)
                    def _():
                        h0 = 2 * (S - 1 - back // NT)
                        cols = pl.ds((tt % NT + 1 - strip) * W2, strip * W2)
                        if back == 0:
                            wr_cols(h0 + h, 1, cols)
                        else:
                            wr_cols(h0, 2, cols)

            issue(0, 0)
            return block(st, hs + i * U, 0, TPI, pbuf[cur], pbuf[cur], stored if final else None)

        return jax.lax.fori_loop(0, NIT, it, st)

    hs = pos // NT
    k0 = kx + 1 + len(head)
    for li, (U, reps) in enumerate(loops):
        st = loop(st, hs, U, reps, k0, li == len(loops) - 1)
        hs += U * reps
        k0 += reps
    pltpu.make_async_copy(obuf, o_hbm, osem.at[0]).wait()


def _run(x, g, b, w, head=(1, 1, 2, 4), loops=((2, 3), (8, 3)), groups=(8,) * 6 + (4, 4, 2, 2),
         tau_w=61, lead=4, spans=(990, 1050), strips=(1, 1, 1, 1, 2, 0, 2)):
    B, S, _ = x.shape
    xt = jnp.transpose(x, (1, 2, 0))
    oshape = (2 * S, NH, B)
    nsem = len(W_STEPS) + 1 + len(head) + sum(reps for _, reps in loops)
    out = pl.pallas_call(
        functools.partial(_body, head=head, loops=loops, groups=groups, tau_w=tau_w, lead=lead, spans=spans,
                          strips=strips),
        in_specs=[pl.BlockSpec(memory_space=pl.ANY)] * 4,
        out_specs=pl.BlockSpec(memory_space=pl.ANY),
        out_shape=jax.ShapeDtypeStruct(oshape, x.dtype),
        scratch_shapes=[
            pltpu.VMEM((S, D, B), BF16),
            pltpu.VMEM(oshape, BF16),
            pltpu.VMEM((D, D), BF16),
            pltpu.VMEM((D,), BF16),
            pltpu.VMEM((D,), BF16),
            pltpu.VMEM((5, D // 2, 128), U32),
            pltpu.VMEM((16, NH, 128), BF16),
            pltpu.VMEM((16, NH // 2, 128), U32),
            pltpu.VMEM((D, T), F32),
            pltpu.VMEM((PROWS, T), BF16),
            pltpu.VMEM((PROWS, T), BF16),
            pltpu.VMEM((8, T), U32),
            pltpu.SemaphoreType.DMA((nsem,)),
            pltpu.SemaphoreType.DMA((1,)),
        ],
        compiler_params=pltpu.CompilerParams(
            vmem_limit_bytes=110 * 1024 * 1024,
            disable_bounds_checks=True,
            disable_semaphore_checks=True,
        ),
    )(xt, g, b, w)
    return jnp.transpose(out.reshape(S, D, B), (2, 0, 1))


@jax.jit
def pallas_standalone__layernorm_linear__sampling_kernel(x, g, b, w):
    return _run(x, g, b, w)
```
